```python
import jax
import jax.numpy as jnp

def _softmax(x, axis=-1):
    return jax.nn.softmax(x, axis=axis)
def _gelu(x):
    return jax.nn.gelu(x, approximate=True)
def _silu(x):
    return jax.nn.silu(x)
def _sigmoid(x):
    return jax.nn.sigmoid(x)
def _layernorm(x, axis=-1, eps=1e-5):
    m = jnp.mean(x, axis=axis, keepdims=True)
    v = jnp.var(x, axis=axis, keepdims=True)
    return (x - m) / jnp.sqrt(v + eps)
def _scatter_add(tgt, idx, src, axis=0):
    return tgt.at[idx].add(src)
def _segment_sum(src, seg, n):
    return jax.ops.segment_sum(src, seg, n)
class _Rng:
    def __init__(self, key):
        self._k = key
    def _next(self):
        self._k, sub = jax.random.split(self._k)
        return sub
    def normal(self, shape):
        return jax.random.normal(self._next(), shape, dtype=jnp.bfloat16)
    def randint(self, lo, hi, shape):
        return jax.random.randint(self._next(), shape, lo, hi, dtype=jnp.int32)
    def uniform(self, shape, lo=0.0, hi=1.0):
        return jax.random.uniform(self._next(), shape, jnp.bfloat16, lo, hi)
    def permutation(self, n):
        return jax.random.permutation(self._next(), n)


kernel_name = 'concat_heads__compressed_kv_cla__gqa_block_cached__decode'

def setup_inputs():
    _rng = _Rng(jax.random.key(int.from_bytes(__import__("os").urandom(4), "little")))
    _w = (lambda a: (lambda t: t.astype(jnp.bfloat16) if jnp.issubdtype(t.dtype, jnp.floating) else t)(jnp.asarray(a)))
    def _A_setup():
        B, H, Sq, Sk, D, M = 2, 32, 1, 4096, 128, 512
        Dc = 4 * D
        return {
            "x": _w((lambda *s: _rng.normal(s) * 0.05)(B, Sq, M)),
            "c_kv": _w((lambda *s: _rng.normal(s) * 0.05)(B, Sk, Dc)),
            "w_q": _w((lambda *s: _rng.normal(s) * 0.05)(M, H, D) * (M ** -0.5)),
            "w_uk": _w((lambda *s: _rng.normal(s) * 0.05)(Dc, H, D) * (Dc ** -0.5)),
            "w_uv": _w((lambda *s: _rng.normal(s) * 0.05)(Dc, H, D) * (Dc ** -0.5)),
            "w_o": _w((lambda *s: _rng.normal(s) * 0.05)(H, D, M) * ((H * D) ** -0.5)),
        }
    _A_in = _A_setup()

    def _B_setup():
        B, Sq, D = 2, 1, 512
        Hq, Hkv, Sk, Dh = 32, 32, 4096, 128
        assert Hq % Hkv == 0, (Hq, Hkv)
        return {
            "x": _w((lambda *s: _rng.normal(s) * 0.05)(B, Sq, D)),
            "k_cache": _w((lambda *s: _rng.normal(s) * 0.05)(B, Hkv, Sk, Dh)),
            "v_cache": _w((lambda *s: _rng.normal(s) * 0.05)(B, Hkv, Sk, Dh)),
            "wq": _w((lambda *s: _rng.normal(s) * 0.05)(D, Hq * Dh) * (D ** -0.5)),
            "wo": _w((lambda *s: _rng.normal(s) * 0.05)(Hq * Dh, D) * ((Hq * Dh) ** -0.5)),
        }
    _B_in = _B_setup()

    return {
        "A_x": _A_in["x"],
        "A_c_kv": _A_in["c_kv"],
        "A_w_q": _A_in["w_q"],
        "A_w_uk": _A_in["w_uk"],
        "A_w_uv": _A_in["w_uv"],
        "A_w_o": _A_in["w_o"],
        "B_x": _B_in["x"],
        "B_k_cache": _B_in["k_cache"],
        "B_v_cache": _B_in["v_cache"],
        "B_wq": _B_in["wq"],
        "B_wo": _B_in["wo"],
    }

def reference(A_x, A_c_kv, A_w_q, A_w_uk, A_w_uv, A_w_o, B_x, B_k_cache, B_v_cache, B_wq, B_wo):
    def _A_ref(x, c_kv, w_q, w_uk, w_uv, w_o):
        B, Sq, M = x.shape[0], x.shape[1], x.shape[2]
        Sk = c_kv.shape[1]
        H, D = w_q.shape[1], w_q.shape[2]
        q = jnp.einsum("bqm,mhd->bhqd", x, w_q)
        k = jnp.einsum("bkc,chd->bhkd", c_kv, w_uk)
        v = jnp.einsum("bkc,chd->bhkd", c_kv, w_uv)
        scores = jnp.einsum("bhqd,bhkd->bhqk", q, k) * (D ** -0.5)
        off = Sk - Sq
        qi = jnp.arange(Sq)[:, None]
        kj = jnp.arange(Sk)[None, :]
        cmask = kj <= (qi + off)
        scores = jnp.where(cmask[None, None], scores, -1e9)
        p = _softmax(scores, axis=-1)
        ctx = jnp.einsum("bhqk,bhkd->bhqd", p, v)
        return jnp.einsum("bhqd,hdm->bqm", ctx, w_o)

    def _B_ref(x, k_cache, v_cache, wq, wo):
        B, Sq, D = x.shape
        Hq, Dh = 32, 128
        Hkv = k_cache.shape[1]
        rep = Hq // Hkv
        q = (lambda x, *d: x.transpose(*d))((x @ wq).reshape(B, Sq, Hq, Dh), 0, 2, 1, 3)
        k = jnp.repeat(k_cache, rep, axis=1)
        v = jnp.repeat(v_cache, rep, axis=1)
        scores = jnp.einsum("bhqd,bhkd->bhqk", q, k) * (Dh ** -0.5)
        p = _softmax(scores, axis=-1)
        o = jnp.einsum("bhqk,bhkd->bhqd", p, v)
        return (lambda x, *d: x.transpose(*d))(o, 0, 2, 1, 3).reshape(B, Sq, Hq * Dh) @ wo

    a = _A_ref(A_x, A_c_kv, A_w_q, A_w_uk, A_w_uv, A_w_o)
    b = _B_ref(B_x, B_k_cache, B_v_cache, B_wq, B_wo)
    return jnp.concatenate([a, b], axis=-1)
```

```python
import jax
import jax.numpy as jnp
from jax import lax
from jax.experimental import pallas as pl
from jax.experimental.pallas import tpu as pltpu

B, H, SK, D, M = 2, 32, 4096, 128, 512
DC = 4 * D
BH = B * H
G = 8
NGROUP = BH // G
KEYS = 256
NJ = SK // KEYS
NW = 8
LAG = 2
NSEM = 8
PAIRS = 16

T_Q = 0
T_U = T_Q + NW
T_C = T_U + NW
T_KV = T_C + NW
T_O = T_KV + NGROUP * NJ
T_END = T_O + NW

SCALE = float(D) ** -0.5
NN = (((1,), (0,)), ((), ()))
NT = (((1,), (1,)), ((), ()))
F32 = jnp.float32
BF16 = jnp.bfloat16


def _dot(a, b, dims=NN):
    return lax.dot_general(a, b, dims, preferred_element_type=F32)


def _iota(shape, dim):
    return lax.broadcasted_iota(jnp.int32, shape, dim)


def _ds(start, size):
    if isinstance(start, int):
        return pl.ds(start, size)
    return pl.ds(pl.multiple_of(start, size), size)


def _kernel(
    xa_hbm, c_hbm, wqa_hbm, wuk_hbm, wuv_hbm, woa_hbm,
    xb_hbm, k_hbm, v_hbm, wqb_hbm, wob_hbm,
    out_ref,
    xa, xb, c, wqa, wuk, wuv, woa, wqb, wob, kbuf, vbuf,
    e_ref, lhs_ref, qb_acc, qb_ref, sa_ref, sb_ref, ob_ref, ctx_ref,
    sems, xsem,
):
    def pieces(t):
        def rows(src, dst, lo, n):
            step = n // PAIRS
            cps = [
                (src.at[_ds(lo + i * step, step)], dst.at[_ds(lo + i * step, step)])
                for i in range(PAIRS)
            ]
            return dst.at[_ds(lo, n)], cps

        if isinstance(t, tuple):
            n, j = t
            slot = n % 2
            res = []
            for src, dst in ((k_hbm, kbuf), (v_hbm, vbuf)):
                cps = [
                    (
                        src.at[n * G + g, _ds(j * KEYS + i * 128, 128)],
                        dst.at[slot, g, _ds(j * KEYS + i * 128, 128)],
                    )
                    for i in range(KEYS // 128)
                    for g in range(G)
                ]
                res.append((dst.at[slot, :, _ds(j * KEYS, KEYS)], cps))
            return res
        part, i = t[0], t[1:]
        raise AssertionError((part, i))

    def weight_pieces(part, i):
        def rows(src, dst, n):
            step = n // PAIRS
            cps = [
                (
                    src.at[_ds(i * n + p * step, step)],
                    dst.at[_ds(i * n + p * step, step)],
                )
                for p in range(PAIRS)
            ]
            return dst.at[_ds(i * n, n)], cps

        if part == "q":
            cps = [
                (
                    wqb_hbm.at[_ds(i * 64 + r * 16, 16), pl.ds(cc * 1024, 1024)],
                    wqb.at[_ds(i * 64 + r * 16, 16), pl.ds(cc * 1024, 1024)],
                )
                for r in range(4)
                for cc in range(4)
            ]
            return [(wqb.at[_ds(i * 64, 64)], cps), rows(wqa_hbm, wqa, 2048)]
        if part == "u":
            return [rows(wuk_hbm, wuk, 2048), rows(wuv_hbm, wuv, 2048)]
        if part == "c":
            return [rows(c_hbm.at[0], c.at[0], 512), rows(c_hbm.at[1], c.at[1], 512)]
        assert part == "o"
        return [rows(woa_hbm, woa, 512), rows(wob_hbm, wob, 512)]

    def start(two, t):
        (_, cps0), (_, cps1) = two
        for (s0, d0), (s1, d1) in zip(cps0, cps1):
            pltpu.make_async_copy(s0, d0, sems.at[t % NSEM, 0]).start(priority=0)
            pltpu.make_async_copy(s1, d1, sems.at[t % NSEM, 1]).start(priority=1)

    def wait(two, t):
        for w, (region, _) in enumerate(two):
            pltpu.make_async_copy(region, region, sems.at[t % NSEM, w]).wait()

    def batch(t):
        if t < T_U:
            return weight_pieces("q", t - T_Q)
        if t < T_C:
            return weight_pieces("u", t - T_U)
        if t < T_KV:
            return weight_pieces("c", t - T_C)
        if t < T_O:
            return pieces(divmod(t - T_KV, NJ))
        return weight_pieces("o", t - T_O)

    def advance(t):
        if t + LAG < T_END:
            start(batch(t + LAG), t + LAG)
        wait(batch(t), t)

    start(batch(0), 0)
    xa_copy = pltpu.make_async_copy(xa_hbm, xa, xsem.at[0])
    xb_copy = pltpu.make_async_copy(xb_hbm, xb, xsem.at[1])
    xa_copy.start()
    xb_copy.start()
    for t in range(1, LAG):
        start(batch(t), t)

    for blk in range(0, 4096, 512):
        hit = _iota((128, 512), 0) == (_iota((128, 512), 1) + blk) // H
        e_ref[:, blk:blk + 512] = jnp.where(hit, 1.0, 0.0).astype(BF16)
    own_head = _iota((BH, 128), 0) % H == _iota((BH, 128), 1) % H

    def keep_own_head(x):
        return jnp.concatenate(
            [
                jnp.where(own_head, x[:, i:i + 128], 0.0).astype(BF16)
                for i in range(0, x.shape[1], 128)
            ],
            axis=1,
        )

    def contract_latent(w_ref, i):
        half = (i % 2) * 2048
        spread = _dot(lhs_ref[i // 2], e_ref[:, half:half + 2048])
        return _dot(keep_own_head(spread), w_ref[i * 2048:(i + 1) * 2048, :])

    xa_copy.wait()
    xb_copy.wait()
    xa_val = xa[...].astype(F32)
    xb_val = xb[...].astype(F32)
    for mb in range(4):
        cols = slice(mb * 128, (mb + 1) * 128)
        lhs_ref[mb] = jnp.concatenate(
            [jnp.broadcast_to(xa_val[b, :, cols], (H, 128)) for b in range(B)], axis=0
        ).astype(BF16)
    xb_rows = jnp.concatenate(
        [jnp.broadcast_to(xb_val[b], (G, M)) for b in range(B)], axis=0
    ).astype(BF16)

    qa = jnp.zeros((BH, D), F32)
    for i in range(NW):
        advance(T_Q + i)
        qa = qa + contract_latent(wqa, i)
        if i % 2:
            rows = slice((i // 2) * 128, (i // 2 + 1) * 128)
            part = _dot(xb_rows[:, rows], wqb[rows, :])
            qb_acc[...] = part if i == 1 else qb_acc[...] + part
    qa = qa.astype(BF16)
    sub = _iota((G, 128), 0)
    for b in range(B):
        for hg in range(H // G):
            q8 = jnp.zeros((G, D), F32)
            for g in range(G):
                h = hg * G + g
                q8 = jnp.where(sub == g, qb_acc[b * G:(b + 1) * G, h * D:(h + 1) * D], q8)
            qb_ref[b * (H // G) + hg] = q8

    for i in range(NW):
        advance(T_U + i)
        if i % 2:
            full = _dot(qa, wuk[(i // 2) * 4096:(i // 2 + 1) * 4096, :], NT)
            lhs_ref[i // 2] = _dot(keep_own_head(full), e_ref[...], NT).astype(BF16)

    ma = jnp.full((BH, 128), -jnp.inf, F32)
    for i in range(NW):
        advance(T_C + i)
        keys = slice(i * 512, (i + 1) * 512)
        s = jnp.concatenate(
            [
                _dot(
                    jnp.concatenate(
                        [lhs_ref[cb, b * H:(b + 1) * H, :] for cb in range(4)], axis=1
                    ),
                    c[b, keys, :],
                    NT,
                )
                for b in range(B)
            ],
            axis=0,
        )
        sa_ref[i] = s
        for k in range(0, 512, 128):
            ma = jnp.maximum(ma, s[:, k:k + 128])
    ma = jnp.max(ma, axis=1, keepdims=True)
    ctx_ref[...] = jnp.zeros(ctx_ref.shape, F32)

    def a_context(i, la):
        p = jnp.exp((sa_ref[i] - ma) * SCALE)
        for k in range(0, 512, 128):
            la = la + p[:, k:k + 128]
        p = p.astype(BF16)
        for b in range(B):
            rows = slice(b * H, (b + 1) * H)
            ctx_ref[rows, :] += _dot(p[rows], c[b, _ds(i * 512, 512), :])
        return la

    sub_keys = _iota((G, KEYS), 0)

    def b_scores(n, j, m):
        q8 = qb_ref[n].astype(BF16)
        s = jnp.zeros((G, KEYS), F32)
        for g in range(G):
            k_tile = kbuf[n % 2, g, _ds(j * KEYS, KEYS), :]
            s = jnp.where(sub_keys == g, _dot(q8, k_tile, NT), s)
        sb_ref[n % 2, j] = s
        for k in range(0, KEYS, 128):
            m = jnp.maximum(m, s[:, k:k + 128])
        return m

    def b_values(n, j, m, l, acc):
        p = jnp.exp((sb_ref[n % 2, j] - m) * SCALE)
        for k in range(0, KEYS, 128):
            l = l + p[:, k:k + 128]
        p = p.astype(BF16)
        for g in range(G):
            v_tile = vbuf[n % 2, g, _ds(j * KEYS, KEYS), :]
            acc = acc + jnp.where(sub == g, _dot(p, v_tile), 0.0)
        return l, acc

    def b_finish(n, l, acc):
        ob_ref[n] = acc / jnp.sum(l, axis=1, keepdims=True)

    def advance_kv(n, j):
        t = T_KV + n * NJ + j
        ahead = n * NJ + j + LAG
        start(pieces((ahead // NJ, ahead % NJ)), t + LAG)
        wait(pieces((n, j)), t)

    neg = jnp.full((G, 128), -jnp.inf, F32)
    zero = jnp.zeros((G, 128), F32)

    def first_group(j, carry):
        m, la = carry
        advance_kv(0, 2 * j)
        m = b_scores(0, 2 * j, m)
        advance_kv(0, 2 * j + 1)
        m = b_scores(0, 2 * j + 1, m)
        return m, a_context(j, la)

    m, la = lax.fori_loop(0, NW, first_group, (neg, jnp.zeros((BH, 128), F32)))
    ctx_lat = ctx_ref[...] / jnp.sum(la, axis=1, keepdims=True)
    for cb in range(4):
        lhs_ref[cb] = ctx_lat[:, cb * 128:(cb + 1) * 128].astype(BF16)

    def step(n, j, m_prev, carry):
        m, l, acc = carry
        m = b_scores(n, j, m)
        l, acc = b_values(n - 1, j, m_prev, l, acc)
        return m, l, acc

    def group(n, m_prev):
        def body(j, carry):
            advance_kv(n, j)
            return step(n, j, m_prev, carry)

        m, l, acc = lax.fori_loop(0, NJ, body, (neg, zero, zero))
        b_finish(n - 1, l, acc)
        return jnp.broadcast_to(jnp.max(m, axis=1, keepdims=True), (G, KEYS))

    m_prev = jnp.broadcast_to(jnp.max(m, axis=1, keepdims=True), (G, KEYS))
    m_prev = lax.fori_loop(1, NGROUP - 1, group, m_prev)

    last = NGROUP - 1

    def last_body(j, carry):
        advance_kv(last, j)
        return step(last, j, m_prev, carry)

    carry = lax.fori_loop(0, NJ - LAG, last_body, (neg, zero, zero))
    for j in range(NJ - LAG, NJ):
        advance(T_KV + last * NJ + j)
        carry = step(last, j, m_prev, carry)
    m, l, acc = carry
    b_finish(last - 1, l, acc)
    m_last = jnp.broadcast_to(jnp.max(m, axis=1, keepdims=True), (G, KEYS))

    l, acc = zero, zero
    ctx = jnp.zeros((BH, D), F32)
    for i in range(NW // 2):
        if i + LAG < NW:
            start(batch(T_O + i + LAG), T_O + i + LAG)
        per = NJ // (NW // 2)
        l, acc = lax.fori_loop(
            i * per, (i + 1) * per,
            lambda j, lc: b_values(last, j, m_last, *lc), (l, acc),
        )
        ctx = ctx + contract_latent(wuv, 2 * i) + contract_latent(wuv, 2 * i + 1)
    b_finish(last, l, acc)

    sub16 = _iota((B * G, 128), 0) % G

    def project(o16, w_ref, i):
        lhs = jnp.concatenate(
            [
                jnp.where(sub16 == (4 * i + u) % G, o16, 0.0).astype(BF16)
                for u in range(4)
            ],
            axis=1,
        )
        return _dot(lhs, w_ref[i * 512:(i + 1) * 512, :])

    out_a = jnp.zeros((B * G, M), F32)
    out_b = jnp.zeros((B * G, M), F32)
    for i in range(NW):
        t = T_O + i + NW // 2 + LAG
        if t < T_END:
            start(batch(t), t)
        wait(batch(T_O + i), T_O + i)
        hg = i // 2
        ctx16 = jnp.concatenate(
            [ctx[b * H + hg * G:b * H + (hg + 1) * G] for b in range(B)], axis=0
        )
        o16 = jnp.concatenate([ob_ref[b * (H // G) + hg] for b in range(B)], axis=0)
        out_a = out_a + project(ctx16, woa, i)
        out_b = out_b + project(o16, wob, i)
    for b in range(B):
        rows = slice(b * G, (b + 1) * G)
        out_ref[b, :, 0:M] = jnp.sum(out_a[rows], axis=0, keepdims=True).astype(BF16)
        out_ref[b, :, M:2 * M] = jnp.sum(out_b[rows], axis=0, keepdims=True).astype(BF16)


@jax.jit
def pallas_concat_heads__compressed_kv_cla__gqa_block_cached__decode_kernel(
    A_x: jax.Array,
    A_c_kv: jax.Array,
    A_w_q: jax.Array,
    A_w_uk: jax.Array,
    A_w_uv: jax.Array,
    A_w_o: jax.Array,
    B_x: jax.Array,
    B_k_cache: jax.Array,
    B_v_cache: jax.Array,
    B_wq: jax.Array,
    B_wo: jax.Array,
):
    assert A_x.shape == B_x.shape == (B, 1, M)
    assert A_c_kv.shape == (B, SK, DC)
    assert B_k_cache.shape == B_v_cache.shape == (B, H, SK, D)
    vmem = pltpu.VMEM
    return pl.pallas_call(
        _kernel,
        in_specs=[pl.BlockSpec(memory_space=pl.ANY)] * 11,
        out_specs=pl.BlockSpec(memory_space=vmem),
        out_shape=jax.ShapeDtypeStruct((B, 1, 2 * M), BF16),
        scratch_shapes=[
            vmem((B, 1, M), BF16),
            vmem((B, 1, M), BF16),
            vmem((B, SK, DC), BF16),
            vmem((M * H, D), BF16),
            vmem((DC * H, D), BF16),
            vmem((DC * H, D), BF16),
            vmem((H * D, M), BF16),
            vmem((M, H * D), BF16),
            vmem((H * D, M), BF16),
            vmem((2, G, SK, D), BF16),
            vmem((2, G, SK, D), BF16),
            vmem((128, 128 * H), BF16),
            vmem((4, BH, 128), BF16),
            vmem((B * G, H * D), F32),
            vmem((NGROUP, G, D), F32),
            vmem((NW, BH, SK // NW), F32),
            vmem((2, NJ, G, KEYS), F32),
            vmem((NGROUP, G, D), F32),
            vmem((BH, DC), F32),
            pltpu.SemaphoreType.DMA((NSEM, 2)),
            pltpu.SemaphoreType.DMA((2,)),
        ],
        compiler_params=pltpu.CompilerParams(
            vmem_limit_bytes=100 * 1024 * 1024,
            disable_bounds_checks=True,
        ),
    )(
        A_x,
        A_c_kv,
        A_w_q.reshape(M * H, D),
        A_w_uk.reshape(DC * H, D),
        A_w_uv.reshape(DC * H, D),
        A_w_o.reshape(H * D, M),
        B_x,
        B_k_cache.reshape(BH, SK, D),
        B_v_cache.reshape(BH, SK, D),
        B_wq,
        B_wo,
    )
```

```python
import jax
import jax.numpy as jnp
from jax import lax
from jax.experimental import pallas as pl
from jax.experimental.pallas import tpu as pltpu

B, H, SK, D, M = 2, 32, 4096, 128, 512
DC = 4 * D
BH = B * H
G = 8
NGROUP = BH // G
KEYS = 256
NJ = SK // KEYS
NW = 8
LAG = 2
NSEM = 8
PAIRS = 16

T_Q = 0
T_U = T_Q + NW
T_C = T_U + NW
T_KV = T_C + NW
T_O = T_KV + NGROUP * NJ
T_END = T_O + NW

SCALE = float(D) ** -0.5
NN = (((1,), (0,)), ((), ()))
NT = (((1,), (1,)), ((), ()))
F32 = jnp.float32
BF16 = jnp.bfloat16


def _dot(a, b, dims=NN):
    return lax.dot_general(a, b, dims, preferred_element_type=F32)


def _iota(shape, dim):
    return lax.broadcasted_iota(jnp.int32, shape, dim)


def _ds(start, size):
    if isinstance(start, int):
        return pl.ds(start, size)
    return pl.ds(pl.multiple_of(start, size), size)


def _kernel(
    xa_hbm, c_hbm, wqa_hbm, wuk_hbm, wuv_hbm, woa_hbm,
    xb_hbm, k_hbm, v_hbm, wqb_hbm, wob_hbm,
    out_ref,
    xa, xb, c, wqa, wuk, wuv, woa, wqb, wob, kbuf, vbuf,
    e_ref, lhs_ref, qb_acc, qb_ref, sa_ref, sb_ref, ob_ref, ctx_ref,
    sems, xsem,
):
    def pieces(t):
        def rows(src, dst, lo, n):
            step = n // PAIRS
            cps = [
                (src.at[_ds(lo + i * step, step)], dst.at[_ds(lo + i * step, step)])
                for i in range(PAIRS)
            ]
            return dst.at[_ds(lo, n)], cps

        if isinstance(t, tuple):
            n, j = t
            slot = n % 2
            res = []
            for src, dst in ((k_hbm, kbuf), (v_hbm, vbuf)):
                cps = [
                    (
                        src.at[n * G + g, _ds(j * KEYS + i * 128, 128)],
                        dst.at[slot, g, _ds(j * KEYS + i * 128, 128)],
                    )
                    for i in range(KEYS // 128)
                    for g in range(G)
                ]
                res.append((dst.at[slot, :, _ds(j * KEYS, KEYS)], cps))
            return res
        part, i = t[0], t[1:]
        raise AssertionError((part, i))

    def weight_pieces(part, i):
        def rows(src, dst, n):
            step = n // PAIRS
            cps = [
                (
                    src.at[_ds(i * n + p * step, step)],
                    dst.at[_ds(i * n + p * step, step)],
                )
                for p in range(PAIRS)
            ]
            return dst.at[_ds(i * n, n)], cps

        if part == "q":
            cps = [
                (
                    wqb_hbm.at[_ds(i * 64 + r * 16, 16), pl.ds(cc * 1024, 1024)],
                    wqb.at[_ds(i * 64 + r * 16, 16), pl.ds(cc * 1024, 1024)],
                )
                for r in range(4)
                for cc in range(4)
            ]
            return [(wqb.at[_ds(i * 64, 64)], cps), rows(wqa_hbm, wqa, 2048)]
        if part == "u":
            return [rows(wuk_hbm, wuk, 2048), rows(wuv_hbm, wuv, 2048)]
        if part == "c":
            return [rows(c_hbm.at[0], c.at[0], 512), rows(c_hbm.at[1], c.at[1], 512)]
        assert part == "o"
        return [rows(woa_hbm, woa, 512), rows(wob_hbm, wob, 512)]

    def start(two, t):
        (_, cps0), (_, cps1) = two
        for (s0, d0), (s1, d1) in zip(cps0, cps1):
            pltpu.make_async_copy(s0, d0, sems.at[t % NSEM, 0]).start(priority=0)
            pltpu.make_async_copy(s1, d1, sems.at[t % NSEM, 1]).start(priority=1)

    def wait(two, t):
        for w, (region, _) in enumerate(two):
            pltpu.make_async_copy(region, region, sems.at[t % NSEM, w]).wait()

    def batch(t):
        if t < T_U:
            return weight_pieces("q", t - T_Q)
        if t < T_C:
            return weight_pieces("u", t - T_U)
        if t < T_KV:
            return weight_pieces("c", t - T_C)
        if t < T_O:
            return pieces(divmod(t - T_KV, NJ))
        return weight_pieces("o", t - T_O)

    def advance(t):
        if t + LAG < T_END:
            start(batch(t + LAG), t + LAG)
        wait(batch(t), t)

    start(batch(0), 0)
    xa_copy = pltpu.make_async_copy(xa_hbm, xa, xsem.at[0])
    xb_copy = pltpu.make_async_copy(xb_hbm, xb, xsem.at[1])
    xa_copy.start()
    xb_copy.start()
    for t in range(1, LAG):
        start(batch(t), t)

    for blk in range(0, 4096, 512):
        hit = _iota((128, 512), 0) == (_iota((128, 512), 1) + blk) // H
        e_ref[:, blk:blk + 512] = jnp.where(hit, 1.0, 0.0).astype(BF16)
    own_head = _iota((BH, 128), 0) % H == _iota((BH, 128), 1) % H

    def keep_own_head(x):
        return jnp.concatenate(
            [
                jnp.where(own_head, x[:, i:i + 128], 0.0).astype(BF16)
                for i in range(0, x.shape[1], 128)
            ],
            axis=1,
        )

    def contract_latent(w_ref, i):
        half = (i % 2) * 2048
        spread = _dot(lhs_ref[i // 2], e_ref[:, half:half + 2048])
        return _dot(keep_own_head(spread), w_ref[i * 2048:(i + 1) * 2048, :])

    xa_copy.wait()
    xb_copy.wait()
    xa_val = xa[...].astype(F32)
    xb_val = xb[...].astype(F32)
    for mb in range(4):
        cols = slice(mb * 128, (mb + 1) * 128)
        lhs_ref[mb] = jnp.concatenate(
            [jnp.broadcast_to(xa_val[b:b + 1, cols], (H, 128)) for b in range(B)], axis=0
        ).astype(BF16)
    xb_rows = jnp.concatenate(
        [jnp.broadcast_to(xb_val[b:b + 1], (G, M)) for b in range(B)], axis=0
    ).astype(BF16)

    qa = jnp.zeros((BH, D), F32)
    for i in range(NW):
        advance(T_Q + i)
        qa = qa + contract_latent(wqa, i)
        if i % 2:
            rows = slice((i // 2) * 128, (i // 2 + 1) * 128)
            part = _dot(xb_rows[:, rows], wqb[rows, :])
            qb_acc[...] = part if i == 1 else qb_acc[...] + part
    qa = qa.astype(BF16)
    sub = _iota((G, 128), 0)
    for b in range(B):
        for hg in range(H // G):
            q8 = jnp.zeros((G, D), F32)
            for g in range(G):
                h = hg * G + g
                q8 = jnp.where(sub == g, qb_acc[b * G:(b + 1) * G, h * D:(h + 1) * D], q8)
            qb_ref[b * (H // G) + hg] = q8

    for i in range(NW):
        advance(T_U + i)
        if i % 2:
            full = _dot(qa, wuk[(i // 2) * 4096:(i // 2 + 1) * 4096, :], NT)
            lhs_ref[i // 2] = _dot(keep_own_head(full), e_ref[...], NT).astype(BF16)

    ma = jnp.full((BH, 128), -jnp.inf, F32)
    for i in range(NW):
        advance(T_C + i)
        keys = slice(i * 512, (i + 1) * 512)
        s = jnp.concatenate(
            [
                _dot(
                    jnp.concatenate(
                        [lhs_ref[cb, b * H:(b + 1) * H, :] for cb in range(4)], axis=1
                    ),
                    c[b, keys, :],
                    NT,
                )
                for b in range(B)
            ],
            axis=0,
        )
        sa_ref[i] = s
        for k in range(0, 512, 128):
            ma = jnp.maximum(ma, s[:, k:k + 128])
    ma = jnp.max(ma, axis=1, keepdims=True)
    ctx_ref[...] = jnp.zeros(ctx_ref.shape, F32)

    def a_context(i, la):
        p = jnp.exp((sa_ref[i] - ma) * SCALE)
        for k in range(0, 512, 128):
            la = la + p[:, k:k + 128]
        p = p.astype(BF16)
        for b in range(B):
            rows = slice(b * H, (b + 1) * H)
            ctx_ref[rows, :] += _dot(p[rows], c[b, _ds(i * 512, 512), :])
        return la

    sub_keys = _iota((G, KEYS), 0)

    def b_scores(n, j, m):
        q8 = qb_ref[n].astype(BF16)
        s = jnp.zeros((G, KEYS), F32)
        for g in range(G):
            k_tile = kbuf[n % 2, g, _ds(j * KEYS, KEYS), :]
            s = jnp.where(sub_keys == g, _dot(q8, k_tile, NT), s)
        sb_ref[n % 2, j] = s
        for k in range(0, KEYS, 128):
            m = jnp.maximum(m, s[:, k:k + 128])
        return m

    def b_values(n, j, m, l, acc):
        p = jnp.exp((sb_ref[n % 2, j] - m) * SCALE)
        for k in range(0, KEYS, 128):
            l = l + p[:, k:k + 128]
        p = p.astype(BF16)
        for g in range(G):
            v_tile = vbuf[n % 2, g, _ds(j * KEYS, KEYS), :]
            acc = acc + jnp.where(sub == g, _dot(p, v_tile), 0.0)
        return l, acc

    def b_finish(n, l, acc):
        ob_ref[n] = acc / jnp.sum(l, axis=1, keepdims=True)

    def advance_kv(n, j):
        t = T_KV + n * NJ + j
        ahead = n * NJ + j + LAG
        start(pieces((ahead // NJ, ahead % NJ)), t + LAG)
        wait(pieces((n, j)), t)

    neg = jnp.full((G, 128), -jnp.inf, F32)
    zero = jnp.zeros((G, 128), F32)

    def first_group(j, carry):
        m, la = carry
        advance_kv(0, 2 * j)
        m = b_scores(0, 2 * j, m)
        advance_kv(0, 2 * j + 1)
        m = b_scores(0, 2 * j + 1, m)
        return m, a_context(j, la)

    m, la = lax.fori_loop(0, NW, first_group, (neg, jnp.zeros((BH, 128), F32)))
    ctx_lat = ctx_ref[...] / jnp.sum(la, axis=1, keepdims=True)
    for cb in range(4):
        lhs_ref[cb] = ctx_lat[:, cb * 128:(cb + 1) * 128].astype(BF16)

    def step(n, j, m_prev, carry):
        m, l, acc = carry
        m = b_scores(n, j, m)
        l, acc = b_values(n - 1, j, m_prev, l, acc)
        return m, l, acc

    def group(n, m_prev):
        def body(j, carry):
            advance_kv(n, j)
            return step(n, j, m_prev, carry)

        m, l, acc = lax.fori_loop(0, NJ, body, (neg, zero, zero))
        b_finish(n - 1, l, acc)
        return jnp.broadcast_to(jnp.max(m, axis=1, keepdims=True), (G, KEYS))

    m_prev = jnp.broadcast_to(jnp.max(m, axis=1, keepdims=True), (G, KEYS))
    m_prev = lax.fori_loop(1, NGROUP - 1, group, m_prev)

    last = NGROUP - 1

    def last_body(j, carry):
        advance_kv(last, j)
        return step(last, j, m_prev, carry)

    carry = lax.fori_loop(0, NJ - LAG, last_body, (neg, zero, zero))
    for j in range(NJ - LAG, NJ):
        advance(T_KV + last * NJ + j)
        carry = step(last, j, m_prev, carry)
    m, l, acc = carry
    b_finish(last - 1, l, acc)
    m_last = jnp.broadcast_to(jnp.max(m, axis=1, keepdims=True), (G, KEYS))

    l, acc = zero, zero
    ctx = jnp.zeros((BH, D), F32)
    for i in range(NW // 2):
        if i + LAG < NW:
            start(batch(T_O + i + LAG), T_O + i + LAG)
        per = NJ // (NW // 2)
        l, acc = lax.fori_loop(
            i * per, (i + 1) * per,
            lambda j, lc: b_values(last, j, m_last, *lc), (l, acc),
        )
        ctx = ctx + contract_latent(wuv, 2 * i) + contract_latent(wuv, 2 * i + 1)
    b_finish(last, l, acc)

    sub16 = _iota((B * G, 128), 0) % G

    def project(o16, w_ref, i):
        lhs = jnp.concatenate(
            [
                jnp.where(sub16 == (4 * i + u) % G, o16, 0.0).astype(BF16)
                for u in range(4)
            ],
            axis=1,
        )
        return _dot(lhs, w_ref[i * 512:(i + 1) * 512, :])

    out_a = jnp.zeros((B * G, M), F32)
    out_b = jnp.zeros((B * G, M), F32)
    for i in range(NW):
        t = T_O + i + NW // 2 + LAG
        if t < T_END:
            start(batch(t), t)
        wait(batch(T_O + i), T_O + i)
        hg = i // 2
        ctx16 = jnp.concatenate(
            [ctx[b * H + hg * G:b * H + (hg + 1) * G] for b in range(B)], axis=0
        )
        o16 = jnp.concatenate([ob_ref[b * (H // G) + hg] for b in range(B)], axis=0)
        out_a = out_a + project(ctx16, woa, i)
        out_b = out_b + project(o16, wob, i)
    out = jnp.concatenate([out_a, out_b], axis=1)
    out_ref[...] = jnp.concatenate(
        [jnp.sum(out[b * G:(b + 1) * G], axis=0, keepdims=True) for b in range(B)], axis=0
    ).astype(BF16)


@jax.jit
def pallas_concat_heads__compressed_kv_cla__gqa_block_cached__decode_kernel(
    A_x: jax.Array,
    A_c_kv: jax.Array,
    A_w_q: jax.Array,
    A_w_uk: jax.Array,
    A_w_uv: jax.Array,
    A_w_o: jax.Array,
    B_x: jax.Array,
    B_k_cache: jax.Array,
    B_v_cache: jax.Array,
    B_wq: jax.Array,
    B_wo: jax.Array,
):
    assert A_x.shape == B_x.shape == (B, 1, M)
    assert A_c_kv.shape == (B, SK, DC)
    assert B_k_cache.shape == B_v_cache.shape == (B, H, SK, D)
    vmem = pltpu.VMEM
    return pl.pallas_call(
        _kernel,
        in_specs=[pl.BlockSpec(memory_space=pl.ANY)] * 11,
        out_specs=pl.BlockSpec(memory_space=vmem),
        out_shape=jax.ShapeDtypeStruct((B, 2 * M), BF16),
        scratch_shapes=[
            vmem((B, M), BF16),
            vmem((B, M), BF16),
            vmem((B, SK, DC), BF16),
            vmem((M * H, D), BF16),
            vmem((DC * H, D), BF16),
            vmem((DC * H, D), BF16),
            vmem((H * D, M), BF16),
            vmem((M, H * D), BF16),
            vmem((H * D, M), BF16),
            vmem((2, G, SK, D), BF16),
            vmem((2, G, SK, D), BF16),
            vmem((128, 128 * H), BF16),
            vmem((4, BH, 128), BF16),
            vmem((B * G, H * D), F32),
            vmem((NGROUP, G, D), F32),
            vmem((NW, BH, SK // NW), F32),
            vmem((2, NJ, G, KEYS), F32),
            vmem((NGROUP, G, D), F32),
            vmem((BH, DC), F32),
            pltpu.SemaphoreType.DMA((NSEM, 2)),
            pltpu.SemaphoreType.DMA((2,)),
        ],
        compiler_params=pltpu.CompilerParams(
            vmem_limit_bytes=100 * 1024 * 1024,
            disable_bounds_checks=True,
        ),
    )(
        A_x.reshape(B, M),
        A_c_kv,
        A_w_q.reshape(M * H, D),
        A_w_uk.reshape(DC * H, D),
        A_w_uv.reshape(DC * H, D),
        A_w_o.reshape(H * D, M),
        B_x.reshape(B, M),
        B_k_cache.reshape(BH, SK, D),
        B_v_cache.reshape(BH, SK, D),
        B_wq,
        B_wo,
    ).reshape(B, 1, 2 * M)
```

```python
import jax
import jax.numpy as jnp
from jax import lax
from jax.experimental import pallas as pl
from jax.experimental.pallas import tpu as pltpu

COMPUTE = True
LAG = 2
PK = [64, 64, 64, 64]
PV = [48, 64, 64, 80]
PN0 = [64, 64, 64, 64, 64, 64, 64, 64]
PN1 = [48, 64, 64, 80, 48, 64, 64, 80]
PW0 = [16, 16, 16, 16, 16, 16, 16, 16]
PW1 = [8, 16, 16, 24, 8, 16, 16, 24]
INTERLEAVE = True

B, H, SK, D, M = 2, 32, 4096, 128, 512
DC = 4 * D
BH = B * H
G = 8
NGROUP = BH // G
KEYS = 256
NJ = SK // KEYS
NW = 8
NSLOT = 8
NS = 4

T_Q = 0
T_U = T_Q + NW
T_C = T_U + NW
T_KV = T_C + NW
T_O = T_KV + NGROUP * NJ
T_END = T_O + NW

SCALE = float(D) ** -0.5
NN = (((1,), (0,)), ((), ()))
NT = (((1,), (1,)), ((), ()))
F32 = jnp.float32
BF16 = jnp.bfloat16


def _dot(a, b, dims=NN):
    return lax.dot_general(a, b, dims, preferred_element_type=F32)


def _iota(shape, dim):
    return lax.broadcasted_iota(jnp.int32, shape, dim)


def _ds(start, size, align):
    if isinstance(start, int):
        return pl.ds(start, size)
    return pl.ds(pl.multiple_of(start, align), size)


def _offsets(sizes):
    return [(sum(sizes[:k]), sizes[k]) for k in range(len(sizes))]


def _kernel(
    xa_hbm, c_hbm, wqa_hbm, wuk_hbm, wuv_hbm, woa_hbm,
    xb_hbm, k_hbm, v_hbm, wqb_hbm, wob_hbm,
    out_ref,
    xa, xb, c, wqa, wuk, wuv, woa, wqb, wob, kbuf, vbuf,
    e_ref, lhs_ref, qlat_ref, qb_ref, sa_ref, la_ref, ob_ref, ctxl_ref, ctx_ref, oa_ref,
    sems, xsem,
):
    def weight(src, dst, sizes):
        per = sum(sizes)
        def stream(i):
            copies = []
            for lo, n in _offsets(sizes):
                for s in range(NS):
                    r = _ds(i * per + lo, n, 8)
                    copies.append((src.at[s, r], dst.at[s, r]))
            return dst.at[:, _ds(i * per, per, per)], copies
        return stream

    def wqb_stream(i):
        copies = []
        for r in range(2):
            for cc in range(4):
                for s in range(NS):
                    idx = (s, _ds(i * 16 + r * 8, 8, 8), pl.ds(cc * 1024, 1024))
                    copies.append((wqb_hbm.at[idx], wqb.at[idx]))
        return wqb.at[:, _ds(i * 16, 16, 16)], copies

    def cache(src, dst, sizes):
        def stream(i):
            n, j, slot = i >> 4, i & (NJ - 1), i & (NSLOT - 1)
            copies = []
            for lo, cnt in _offsets(sizes):
                for g in range(G):
                    copies.append((src.at[n * G + g, _ds(j * KEYS + lo, cnt, 8)], dst.at[slot, g, pl.ds(lo, cnt)]))
            return dst.at[slot], copies
        return stream

    parts = (
        (T_Q, T_U, wqb_stream, weight(wqa_hbm, wqa, PN1)),
        (T_U, T_C, weight(wuk_hbm, wuk, PN0), weight(wuv_hbm, wuv, PN1)),
        (T_C, T_KV, weight(c_hbm.at[0], c.at[0], PW0), weight(c_hbm.at[1], c.at[1], PW1)),
        (T_KV, T_O, cache(k_hbm, kbuf, PK), cache(v_hbm, vbuf, PV)),
        (T_O, T_END, weight(woa_hbm, woa, PW0), weight(wob_hbm, wob, PW1)),
    )

    def start(part, t, quarter=None):
        first, _, *streams = parts[part]
        lists = [stream(t - first)[1] for stream in streams]
        n = len(lists[0])
        assert len(lists[1]) == n
        lo, hi = (0, n) if quarter is None else (quarter * n // 4, (quarter + 1) * n // 4)
        for k in range(lo, hi):
            for prio in range(2):
                src, dst = lists[prio][k]
                pltpu.make_async_copy(src, dst, sems.at[t & (NSLOT - 1), prio]).start(priority=prio)

    def wait(part, t):
        first, _, *streams = parts[part]
        for prio, stream in enumerate(streams):
            filled = stream(t - first)[0]
            pltpu.make_async_copy(filled, filled, sems.at[t & (NSLOT - 1), prio]).wait()

    def run(part, body, carry, lo=None, hi=None):
        first, end = parts[part][:2]
        def make(ahead_part):
            def step(t, carry):
                def issue(q):
                    if ahead_part is None:
                        return
                    if INTERLEAVE:
                        start(ahead_part, t + LAG, q)
                    elif q == 0:
                        start(ahead_part, t + LAG)
                issue(0)
                wait(part, t)
                if not COMPUTE:
                    for q in range(1, 4):
                        issue(q)
                    return carry
                return body(t - first, carry, issue)
            return step
        carry = lax.fori_loop(first, end - LAG, make(part), carry)
        return lax.fori_loop(end - LAG, end, make(part + 1 if part + 1 < len(parts) else None), carry)

    start(0, 0)
    xa_copy = pltpu.make_async_copy(xa_hbm, xa, xsem.at[0])
    xb_copy = pltpu.make_async_copy(xb_hbm, xb, xsem.at[1])
    xa_copy.start()
    xb_copy.start()

    if COMPUTE:
        def fill_e(blk, carry):
            hit = _iota((128, 512), 0) == (_iota((128, 512), 1) >> 5) + blk * (512 // H)
            e_ref[blk] = jnp.where(hit, 1.0, 0.0).astype(BF16)
            return carry
        lax.fori_loop(0, NW, fill_e, None)
    lax.fori_loop(1, LAG, lambda t, _: start(0, t), None)
    xa_copy.wait()
    xb_copy.wait()

    if not COMPUTE:
        for part in range(5):
            run(part, None, None)
        out_ref[...] = jnp.zeros(out_ref.shape, out_ref.dtype)
        return

    own_head = (_iota((NS * BH, 128), 0) & (H - 1)) == (_iota((NS * BH, 128), 1) & (H - 1))

    def keep_own_head(x):
        return jnp.concatenate(
            [jnp.where(own_head, x[:, i:i + 128], 0.0).astype(BF16) for i in range(0, x.shape[1], 128)],
            axis=1,
        )

    def contract_latent(w_ref, i, issue):
        spread = keep_own_head(_dot(lhs_ref[...], e_ref[i]))
        issue(1)
        acc = None
        for s in range(NS):
            part = _dot(spread[s * BH:(s + 1) * BH], w_ref[s, _ds(i * 512, 512, 512), :])
            acc = part if acc is None else acc + part
            if s == 1:
                issue(2)
        issue(3)
        return acc

    xa_val = xa[...].astype(F32)
    xb_val = xb[...].astype(F32)
    for s in range(NS):
        for b in range(B):
            lhs_ref[s * BH + b * H:s * BH + (b + 1) * H, :] = jnp.broadcast_to(
                xa_val[b:b + 1, s * 128:(s + 1) * 128], (H, 128)).astype(BF16)
    xb_rows = jnp.concatenate(
        [jnp.broadcast_to(xb_val[b:b + 1], (G, M)) for b in range(B)], axis=0
    ).astype(BF16)
    sub = _iota((G, 128), 0)
    sub16 = _iota((B * G, 128), 0) & (G - 1)
    qb_ref[...] = jnp.zeros(qb_ref.shape, F32)
    qlat_ref[...] = jnp.zeros(qlat_ref.shape, F32)
    ctxl_ref[...] = jnp.zeros(ctxl_ref.shape, F32)
    ctx_ref[...] = jnp.zeros(ctx_ref.shape, F32)
    la_ref[...] = jnp.zeros(la_ref.shape, F32)

    qa = run(0, lambda i, qa, issue: qa + contract_latent(wqa, i, issue), jnp.zeros((BH, D), F32)).astype(BF16)

    def absorb(i, carry, issue):
        full = jnp.concatenate(
            [_dot(qa, wuk[s, _ds(i * 512, 512, 512), :], NT) for s in range(NS)], axis=0)
        issue(1)
        qlat_ref[...] += _dot(keep_own_head(full), e_ref[i], NT)
        issue(2)
        cols = _ds(i * 512, 512, 512)
        full = None
        for s in range(NS):
            part = _dot(xb_rows[:, s * 128:(s + 1) * 128], wqb[s, :, cols])
            full = part if full is None else full + part
        issue(3)
        q16 = qb_ref[i >> 1]
        for u in range(4):
            q16 = jnp.where(sub16 == (i & 1) * 4 + u, full[:, u * D:(u + 1) * D], q16)
        qb_ref[i >> 1] = q16
        return carry

    run(1, absorb, None)
    qlat = [
        jnp.concatenate([qlat_ref[s * BH + b * H:s * BH + (b + 1) * H, :] for s in range(NS)], axis=1).astype(BF16)
        for b in range(B)
    ]

    def latents(b, i):
        return jnp.concatenate([c[b, s, _ds(i * 128, 128, 128), :] for s in range(NS)], axis=0)

    def a_scores(i, ma, issue):
        s0 = _dot(qlat[0], latents(0, i), NT)
        issue(1)
        s1 = _dot(qlat[1], latents(1, i), NT)
        issue(2)
        s = jnp.concatenate([s0, s1], axis=0)
        sa_ref[i] = s
        issue(3)
        for k in range(0, 512, 128):
            ma = jnp.maximum(ma, s[:, k:k + 128])
        return ma

    ma = run(2, a_scores, jnp.full((BH, 128), -jnp.inf, F32))
    ma = jnp.broadcast_to(jnp.max(ma, axis=1, keepdims=True), (BH, 128))

    def a_context(i):
        s = sa_ref[i]
        ps = [jnp.exp((s[:, k:k + 128] - ma) * SCALE) for k in range(0, 512, 128)]
        la_ref[...] += (ps[0] + ps[1]) + (ps[2] + ps[3])
        p = jnp.concatenate(ps, axis=1).astype(BF16)
        for b in range(B):
            r = slice(b * H, (b + 1) * H)
            ctxl_ref[r, :] += _dot(p[r], latents(b, i))

    def a_normalize():
        ctx_lat = ctxl_ref[...] / jnp.sum(la_ref[...], axis=1, keepdims=True)
        for s in range(NS):
            lhs_ref[s * BH:(s + 1) * BH, :] = ctx_lat[:, s * 128:(s + 1) * 128].astype(BF16)

    sub_keys = _iota((G, KEYS), 0)

    def b_step(i, carry, issue):
        n, j, slot = i >> 4, i & (NJ - 1), i & (NSLOT - 1)
        hg, r = n & (H // G - 1), _ds((n >> 2) * G, G, G)
        fresh = j == 0
        m_old = jnp.where(fresh, -jnp.inf, carry[0])
        l_old = jnp.where(fresh, 0.0, carry[1])
        acc = jnp.where(fresh, 0.0, carry[2])
        q8 = qb_ref[hg, r, :].astype(BF16)
        s = jnp.zeros((G, KEYS), F32)
        for g in range(G):
            s = jnp.where(sub_keys == g, _dot(q8, kbuf[slot, g], NT), s)
        issue(1)
        halves = [s[:, k:k + 128] for k in range(0, KEYS, 128)]
        m = jnp.maximum(m_old, jnp.max(jnp.maximum(*halves), axis=1, keepdims=True))
        alpha = jnp.exp((m_old - m) * SCALE)
        ps = [jnp.exp((x - m) * SCALE) for x in halves]
        l = alpha * l_old + (ps[0] + ps[1])
        p = jnp.concatenate(ps, axis=1).astype(BF16)
        acc = alpha * acc
        issue(2)
        for g in range(G):
            acc = acc + jnp.where(sub == g, _dot(p, vbuf[slot, g]), 0.0)
        issue(3)

        @pl.when(j == NJ - 1)
        def _():
            ob_ref[hg, r, :] = acc / jnp.sum(l, axis=1, keepdims=True)

        @pl.when(jnp.logical_and(i < 2 * NJ, (i & 1) == 0))
        def _():
            @pl.when(i < NJ)
            def _():
                a_context(i >> 1)

            @pl.when(i == NJ)
            def _():
                a_normalize()

            @pl.when(i >= NJ)
            def _():
                ctx_ref[...] += contract_latent(wuv, (i - NJ) >> 1, lambda q: None)

        return m, l, acc

    zero = jnp.zeros((G, 128), F32)
    run(3, b_step, (zero, zero, zero))

    for hg in range(H // G):
        oa_ref[hg] = jnp.concatenate(
            [ctx_ref[b * H + hg * G:b * H + (hg + 1) * G, :] for b in range(B)], axis=0
        )

    def project(o_ref, w_ref, i):
        acc = None
        for s in range(NS):
            lhs = jnp.where(sub16 == i, o_ref[s], 0.0).astype(BF16)
            part = _dot(lhs, w_ref[s, _ds(i * 128, 128, 128), :])
            acc = part if acc is None else acc + part
        return acc

    def outputs(i, carry, issue):
        out_a = carry[0] + project(oa_ref, woa, i)
        issue(1)
        issue(2)
        out_b = carry[1] + project(ob_ref, wob, i)
        issue(3)
        return out_a, out_b

    out = jnp.zeros((B * G, M), F32)
    out = jnp.concatenate(run(4, outputs, (out, out)), axis=1)
    out_ref[...] = jnp.concatenate(
        [jnp.sum(out[b * G:(b + 1) * G], axis=0, keepdims=True) for b in range(B)], axis=0
    ).astype(BF16)


@jax.jit
def pallas_concat_heads__compressed_kv_cla__gqa_block_cached__decode_kernel(
    A_x, A_c_kv, A_w_q, A_w_uk, A_w_uv, A_w_o, B_x, B_k_cache, B_v_cache, B_wq, B_wo,
):
    vmem = pltpu.VMEM
    return pl.pallas_call(
        _kernel,
        in_specs=[pl.BlockSpec(memory_space=pl.ANY)] * 11,
        out_specs=pl.BlockSpec(memory_space=vmem),
        out_shape=jax.ShapeDtypeStruct((B, 2 * M), BF16),
        scratch_shapes=[
            vmem((B, M), BF16),
            vmem((B, M), BF16),
            vmem((B, NS, SK // NS, DC), BF16),
            vmem((NS, M * H // NS, D), BF16),
            vmem((NS, DC * H // NS, D), BF16),
            vmem((NS, DC * H // NS, D), BF16),
            vmem((NS, H * D // NS, M), BF16),
            vmem((NS, M // NS, H * D), BF16),
            vmem((NS, H * D // NS, M), BF16),
            vmem((NSLOT, G, KEYS, D), BF16),
            vmem((NSLOT, G, KEYS, D), BF16),
            vmem((NW, 128, 512), BF16),
            vmem((NS * BH, 128), BF16),
            vmem((NS * BH, 128), F32),
            vmem((H // G, B * G, D), F32),
            vmem((NW, BH, SK // NW), F32),
            vmem((BH, 128), F32),
            vmem((H // G, B * G, D), F32),
            vmem((BH, DC), F32),
            vmem((BH, D), F32),
            vmem((H // G, B * G, D), F32),
            pltpu.SemaphoreType.DMA((NSLOT, 2)),
            pltpu.SemaphoreType.DMA((2,)),
        ],
        compiler_params=pltpu.CompilerParams(
            vmem_limit_bytes=100 * 1024 * 1024,
            disable_bounds_checks=True,
        ),
    )(
        A_x.reshape(B, M),
        A_c_kv.reshape(B, NS, SK // NS, DC),
        A_w_q.reshape(NS, M * H // NS, D),
        A_w_uk.reshape(NS, DC * H // NS, D),
        A_w_uv.reshape(NS, DC * H // NS, D),
        A_w_o.reshape(NS, H * D // NS, M),
        B_x.reshape(B, M),
        B_k_cache.reshape(BH, SK, D),
        B_v_cache.reshape(BH, SK, D),
        B_wq.reshape(NS, M // NS, H * D),
        B_wo.reshape(NS, H * D // NS, M),
    ).reshape(B, 1, 2 * M)
```

```python
import jax
import jax.numpy as jnp
from jax import lax
from jax.experimental import pallas as pl
from jax.experimental.pallas import tpu as pltpu

B, H, SK, D, M = 2, 32, 4096, 128, 512
DC = 4 * D
BH = B * H
G = 8
KEYS = 256
NJ = SK // KEYS
NS = 4
NW = 8
LAG = 3
NSLOT = 4

T_Q = 0
T_U = T_Q + NW
T_C = T_U + NW
T_KV = T_C + NW
T_O = T_KV + BH // G * NJ
T_END = T_O + NW

CUT_CACHE = ((64, 64, 64, 64), (80, 48, 80, 48))
CUT_NARROW = ((64,) * 8, (56, 72) * 4)
CUT_WIDE = ((8, 24) * 4, (16,) * 8)

SCALE = float(D) ** -0.5
NN = (((1,), (0,)), ((), ()))
NT = (((1,), (1,)), ((), ()))
F32 = jnp.float32
BF16 = jnp.bfloat16


def _dot(a, b, dims=NN):
    return lax.dot_general(a, b, dims, preferred_element_type=F32)


def _iota(shape, dim):
    return lax.broadcasted_iota(jnp.int32, shape, dim)


def _ds(start, size, align):
    if isinstance(start, int):
        return pl.ds(start, size)
    return pl.ds(pl.multiple_of(start, align), size)


def _cuts(sizes):
    return [(sum(sizes[:k]), size) for k, size in enumerate(sizes)]


def _kernel(
    xa_hbm, c_hbm, wqa_hbm, wuk_hbm, wuv_hbm, woa_hbm,
    xb_hbm, k_hbm, v_hbm, wqb_hbm, wob_hbm,
    out_ref,
    xa, xb, c, wqa, wuk, wuv, woa, wqb, wob, kbuf, vbuf,
    e_ref, lhs_ref, qlat_ref, qb_ref, sa_ref, la_ref, ctxl_ref, ctx_ref, oa_ref, ob_ref,
    sems, small_sems,
):
    def weight(src, dst, sizes):
        rows = sum(sizes)

        def stream(i):
            pairs = []
            for lo, size in _cuts(sizes):
                r = _ds(i * rows + lo, size, 8)
                pairs += [(src.at[s, r], dst.at[s, r]) for s in range(NS)]
            return dst.at[:, _ds(i * rows, rows, rows)], pairs

        return stream

    def wqb_stream(i):
        pairs = []
        for lo in (0, 8):
            for col in range(0, H * D, 1024):
                idx = (_ds(i * 16 + lo, 8, 8), pl.ds(col, 1024))
                pairs += [(wqb_hbm.at[s, *idx], wqb.at[s, *idx]) for s in range(NS)]
        return wqb.at[:, _ds(i * 16, 16, 16)], pairs

    def cache(src, dst, sizes):
        def stream(i):
            n, j, slot = i >> 4, i & (NJ - 1), i & (NSLOT - 1)
            pairs = []
            for lo, size in _cuts(sizes):
                keys = _ds(j * KEYS + lo, size, 8)
                pairs += [
                    (src.at[n * G + g, keys], dst.at[slot, g, pl.ds(lo, size)])
                    for g in range(G)
                ]
            return dst.at[slot], pairs

        return stream

    def both(make, first, second, sizes):
        return make(*first, sizes[0]), make(*second, sizes[1])

    parts = (
        (T_Q, T_U, (wqb_stream, weight(wqa_hbm, wqa, CUT_NARROW[1]))),
        (T_U, T_C, both(weight, (wuk_hbm, wuk), (wuv_hbm, wuv), CUT_NARROW)),
        (T_C, T_KV, both(weight, (c_hbm.at[0], c.at[0]), (c_hbm.at[1], c.at[1]), CUT_WIDE)),
        (T_KV, T_O, both(cache, (k_hbm, kbuf), (v_hbm, vbuf), CUT_CACHE)),
        (T_O, T_END, both(weight, (woa_hbm, woa), (wob_hbm, wob), CUT_WIDE)),
    )

    def start(part, t):
        first, _, streams = parts[part]
        sem = sems.at[t & (NSLOT - 1)]
        for two in zip(*(stream(t - first)[1] for stream in streams), strict=True):
            for priority, (src, dst) in enumerate(two):
                pltpu.make_async_copy(src, dst, sem).start(priority=priority)

    def wait(part, t):
        first, _, streams = parts[part]
        for stream in streams:
            filled = stream(t - first)[0]
            pltpu.make_async_copy(filled, filled, sems.at[t & (NSLOT - 1)]).wait()

    def run(part, body, carry):
        first, end, _ = parts[part]

        def step(t, carry):
            pl.when(t + LAG < end)(lambda: start(part, t + LAG))
            pl.when(t + LAG >= end)(lambda: start(part + 1, t + LAG))
            wait(part, t)
            return body(t - first, carry)

        return lax.fori_loop(first, end, step, carry)

    start(0, 0)
    xa_copy = pltpu.make_async_copy(xa_hbm, xa, small_sems.at[0])
    xb_copy = pltpu.make_async_copy(xb_hbm, xb, small_sems.at[1])
    xa_copy.start()
    xb_copy.start()
    lax.fori_loop(1, LAG, lambda t, _: start(0, t), None)

    ones = jnp.where(_iota((16, 512), 0) == _iota((16, 512), 1) >> 5, 1.0, 0.0)

    def fill_e(i, carry):
        e_ref[i] = jnp.zeros((128, 512), BF16)
        e_ref[i, _ds(i * 16, 16, 16), :] = ones.astype(BF16)
        return carry

    lax.fori_loop(0, NW, fill_e, None)
    own_head = _iota((NS * BH, 128), 0) & (H - 1) == _iota((NS * BH, 128), 1) & (H - 1)

    def keep_own_head(x):
        return jnp.concatenate(
            [
                jnp.where(own_head, x[:, k:k + 128], 0.0).astype(BF16)
                for k in range(0, x.shape[1], 128)
            ],
            axis=1,
        )

    def contract_latent(w_ref, i):
        spread = keep_own_head(_dot(lhs_ref[...], e_ref[i]))
        return sum(
            _dot(spread[s * BH:(s + 1) * BH], w_ref[s, _ds(i * 512, 512, 512), :])
            for s in range(NS)
        )

    for ref in (qb_ref, qlat_ref, la_ref, ctxl_ref, ctx_ref):
        ref[...] = jnp.zeros(ref.shape, F32)
    xa_copy.wait()
    xb_copy.wait()
    xa_val = xa[...].astype(F32)
    xb_val = xb[...].astype(F32)
    for s in range(NS):
        for b in range(B):
            x = xa_val[b:b + 1, s * 128:(s + 1) * 128]
            lhs_ref[pl.ds(s * BH + b * H, H), :] = jnp.broadcast_to(x, (H, 128)).astype(BF16)
    xb_rows = jnp.concatenate(
        [jnp.broadcast_to(xb_val[b:b + 1], (G, M)) for b in range(B)], axis=0
    ).astype(BF16)
    head_row = _iota((B * G, 128), 0) & (G - 1)

    qa = run(0, lambda i, qa: qa + contract_latent(wqa, i), jnp.zeros((BH, D), F32))
    qa = qa.astype(BF16)

    def queries(i, carry):
        full = jnp.concatenate(
            [_dot(qa, wuk[s, _ds(i * 512, 512, 512), :], NT) for s in range(NS)], axis=0
        )
        qlat_ref[...] += _dot(keep_own_head(full), e_ref[i], NT)
        cols = _ds(i * 512, 512, 512)
        full = sum(
            _dot(xb_rows[:, s * 128:(s + 1) * 128], wqb[s, :, cols]) for s in range(NS)
        )
        q16 = qb_ref[i >> 1]
        for u in range(4):
            q16 = jnp.where(head_row == (i & 1) * 4 + u, full[:, u * D:(u + 1) * D], q16)
        qb_ref[i >> 1] = q16
        return carry

    run(1, queries, None)

    qlat = [
        jnp.concatenate(
            [qlat_ref[pl.ds(s * BH + b * H, H), :] for s in range(NS)], axis=1
        ).astype(BF16)
        for b in range(B)
    ]

    def latents(b, i):
        return jnp.concatenate(
            [c[b, s, _ds(i * 128, 128, 128), :] for s in range(NS)], axis=0
        )

    def a_scores(i, m):
        s = jnp.concatenate([_dot(qlat[b], latents(b, i), NT) for b in range(B)], axis=0)
        sa_ref[i] = s
        for k in range(0, 512, 128):
            m = jnp.maximum(m, s[:, k:k + 128])
        return m

    ma = run(2, a_scores, jnp.full((BH, 128), -jnp.inf, F32))
    ma = jnp.broadcast_to(jnp.max(ma, axis=1, keepdims=True), (BH, 128))

    def a_context(i):
        s = sa_ref[i]
        ps = [jnp.exp((s[:, k:k + 128] - ma) * SCALE) for k in range(0, 512, 128)]
        la_ref[...] += (ps[0] + ps[1]) + (ps[2] + ps[3])
        p = jnp.concatenate(ps, axis=1).astype(BF16)
        for b in range(B):
            rows = slice(b * H, (b + 1) * H)
            ctxl_ref[rows, :] += _dot(p[rows], latents(b, i))

    def a_normalize():
        ctx_lat = ctxl_ref[...] / jnp.sum(la_ref[...], axis=1, keepdims=True)
        for s in range(NS):
            lhs_ref[pl.ds(s * BH, BH), :] = ctx_lat[:, s * 128:(s + 1) * 128].astype(BF16)

    def a_values(i):
        ctx_ref[...] += contract_latent(wuv, i)

    row = _iota((G, 128), 0)
    row_keys = _iota((G, KEYS), 0)

    def b_step(i, carry):
        n, j, slot = i >> 4, i & (NJ - 1), i & (NSLOT - 1)
        block, rows = n & (H // G - 1), _ds((n >> 2) * G, G, G)
        m_old = jnp.where(j == 0, -jnp.inf, carry[0])
        l_old = jnp.where(j == 0, 0.0, carry[1])
        acc = jnp.where(j == 0, 0.0, carry[2])
        q = qb_ref[block, rows, :].astype(BF16)
        s = jnp.zeros((G, KEYS), F32)
        for g in range(G):
            s = jnp.where(row_keys == g, _dot(q, kbuf[slot, g], NT), s)
        halves = [s[:, :128], s[:, 128:]]
        m = jnp.maximum(m_old, jnp.max(jnp.maximum(*halves), axis=1, keepdims=True))
        alpha = jnp.exp((m_old - m) * SCALE)
        ps = [jnp.exp((half - m) * SCALE) for half in halves]
        l = alpha * l_old + (ps[0] + ps[1])
        p = jnp.concatenate(ps, axis=1).astype(BF16)
        acc = alpha * acc
        for g in range(G):
            acc = acc + jnp.where(row == g, _dot(p, vbuf[slot, g]), 0.0)

        @pl.when(j == NJ - 1)
        def _():
            ob_ref[block, rows, :] = acc / jnp.sum(l, axis=1, keepdims=True)

        @pl.when(jnp.logical_and(i < 4 * NW, i & 1 == 0))
        def _():
            pl.when(i < 2 * NW)(lambda: a_context(i >> 1))
            pl.when(i == 2 * NW)(a_normalize)
            pl.when(i >= 2 * NW)(lambda: a_values((i >> 1) - NW))

        return m, l, acc

    zero = jnp.zeros((G, 128), F32)
    run(3, b_step, (zero, zero, zero))

    for s in range(NS):
        oa_ref[s] = jnp.concatenate(
            [ctx_ref[pl.ds(b * H + s * G, G), :] for b in range(B)], axis=0
        )

    def project(s, i, out):
        rows = _ds(i * D, D, D)
        return tuple(
            acc + _dot(jnp.where(head_row == i, o_ref[s], 0.0).astype(BF16), w_ref[s, rows, :])
            for acc, o_ref, w_ref in zip(out, (oa_ref, ob_ref), (woa, wob))
        )

    def start_last():
        for s in range(NS):
            for two in zip(*map(_cuts, CUT_WIDE)):
                for priority, (src, dst) in enumerate(((woa_hbm, woa), (wob_hbm, wob))):
                    lo, size = two[priority]
                    r = pl.ds((NW - 1) * D + lo, size)
                    copy = pltpu.make_async_copy(src.at[s, r], dst.at[s, r], small_sems.at[s])
                    copy.start(priority=priority)

    def outputs(i, out):
        pl.when(i + LAG < NW - 1)(lambda: start(4, T_O + i + LAG))
        pl.when(i + LAG == NW - 1)(start_last)
        wait(4, T_O + i)
        for s in range(NS):
            out = project(s, i, out)
        return out

    out = lax.fori_loop(0, NW - 1, outputs, (jnp.zeros((B * G, M), F32),) * 2)
    for s in range(NS):
        for dst in (woa, wob):
            filled = dst.at[s, pl.ds((NW - 1) * D, D)]
            pltpu.make_async_copy(filled, filled, small_sems.at[s]).wait()
        out = project(s, NW - 1, out)
    out = jnp.concatenate(out, axis=1)
    out_ref[...] = jnp.concatenate(
        [jnp.sum(out[b * G:(b + 1) * G], axis=0, keepdims=True) for b in range(B)], axis=0
    ).astype(BF16)


@jax.jit
def pallas_concat_heads__compressed_kv_cla__gqa_block_cached__decode_kernel(
    A_x: jax.Array,
    A_c_kv: jax.Array,
    A_w_q: jax.Array,
    A_w_uk: jax.Array,
    A_w_uv: jax.Array,
    A_w_o: jax.Array,
    B_x: jax.Array,
    B_k_cache: jax.Array,
    B_v_cache: jax.Array,
    B_wq: jax.Array,
    B_wo: jax.Array,
):
    assert A_x.shape == B_x.shape == (B, 1, M)
    assert A_c_kv.shape == (B, SK, DC)
    assert A_w_q.shape == (M, H, D) and A_w_o.shape == (H, D, M)
    assert A_w_uk.shape == A_w_uv.shape == (DC, H, D)
    assert B_k_cache.shape == B_v_cache.shape == (B, H, SK, D)
    assert B_wq.shape == (M, H * D) and B_wo.shape == (H * D, M)
    vmem = pltpu.VMEM
    out = pl.pallas_call(
        _kernel,
        in_specs=[pl.BlockSpec(memory_space=pl.ANY)] * 11,
        out_specs=pl.BlockSpec(memory_space=vmem),
        out_shape=jax.ShapeDtypeStruct((B, 2 * M), BF16),
        scratch_shapes=[
            vmem((B, M), BF16),
            vmem((B, M), BF16),
            vmem((B, NS, SK // NS, DC), BF16),
            vmem((NS, M * H // NS, D), BF16),
            vmem((NS, DC * H // NS, D), BF16),
            vmem((NS, DC * H // NS, D), BF16),
            vmem((NS, H * D // NS, M), BF16),
            vmem((NS, M // NS, H * D), BF16),
            vmem((NS, H * D // NS, M), BF16),
            vmem((NSLOT, G, KEYS, D), BF16),
            vmem((NSLOT, G, KEYS, D), BF16),
            vmem((NW, 128, 512), BF16),
            vmem((NS * BH, 128), BF16),
            vmem((NS * BH, 128), F32),
            vmem((H // G, B * G, D), F32),
            vmem((NW, BH, SK // NW), F32),
            vmem((BH, 128), F32),
            vmem((BH, DC), F32),
            vmem((BH, D), F32),
            vmem((H // G, B * G, D), F32),
            vmem((H // G, B * G, D), F32),
            pltpu.SemaphoreType.DMA((NSLOT,)),
            pltpu.SemaphoreType.DMA((NS,)),
        ],
        compiler_params=pltpu.CompilerParams(
            vmem_limit_bytes=64 * 1024 * 1024,
            disable_bounds_checks=True,
            disable_semaphore_checks=True,
        ),
    )(
        A_x.reshape(B, M),
        A_c_kv.reshape(B, NS, SK // NS, DC),
        A_w_q.reshape(NS, M * H // NS, D),
        A_w_uk.reshape(NS, DC * H // NS, D),
        A_w_uv.reshape(NS, DC * H // NS, D),
        A_w_o.reshape(NS, H * D // NS, M),
        B_x.reshape(B, M),
        B_k_cache.reshape(BH, SK, D),
        B_v_cache.reshape(BH, SK, D),
        B_wq.reshape(NS, M // NS, H * D),
        B_wo.reshape(NS, H * D // NS, M),
    )
    return out.reshape(B, 1, 2 * M)
```

```python
import jax
import jax.numpy as jnp
from jax import lax
from jax.experimental import pallas as pl
from jax.experimental.pallas import tpu as pltpu

B, H, SK, D, M = 2, 32, 4096, 128, 512
DC = 4 * D
BH = B * H
G = 8
KEYS = 256
NJ = SK // KEYS
NS = 4
NW = 8
LAG = 3
NSLOT = 4

T_Q = 0
T_U = T_Q + NW
T_C = T_U + NW
T_KV = T_C + NW
T_O = T_KV + BH // G * NJ
T_END = T_O + NW

CUT_CACHE = ((64, 64, 64, 64), (80, 48, 80, 48))
CUT_NARROW = ((128,) * 4, (64,) * 8)
CUT_WIDE = ((32,) * 4, (16,) * 8)

SCALE = float(D) ** -0.5
NN = (((1,), (0,)), ((), ()))
NT = (((1,), (1,)), ((), ()))
F32 = jnp.float32
BF16 = jnp.bfloat16


def _dot(a, b, dims=NN):
    return lax.dot_general(a, b, dims, preferred_element_type=F32)


def _iota(shape, dim):
    return lax.broadcasted_iota(jnp.int32, shape, dim)


def _ds(start, size, align):
    if isinstance(start, int):
        return pl.ds(start, size)
    return pl.ds(pl.multiple_of(start, align), size)


def _cuts(sizes):
    return [(sum(sizes[:k]), size) for k, size in enumerate(sizes)]


def _start_interleaved(lists, sem):
    order = sorted(
        ((k + 0.5 * (1 - priority)) / len(pairs), priority, k)
        for priority, pairs in enumerate(lists)
        for k in range(len(pairs))
    )
    for _, priority, k in order:
        pltpu.make_async_copy(*lists[priority][k], sem).start(priority=priority)


def _kernel(
    xa_hbm, c_hbm, wqa_hbm, wuk_hbm, wuv_hbm, woa_hbm,
    xb_hbm, k_hbm, v_hbm, wqb_hbm, wob_hbm,
    out_ref,
    xa, xb, c, wqa, wuk, wuv, woa, wqb, wob, kbuf, vbuf,
    e_ref, lhs_ref, qlat_ref, qb_ref, sa_ref, la_ref, ctxl_ref, ctx_ref, oa_ref, ob_ref,
    sems, small_sems,
):
    def weight(src, dst, sizes):
        rows = sum(sizes)

        def stream(i):
            cuts = [_ds(i * rows + lo, size, size) for lo, size in _cuts(sizes)]
            pairs = [(src.at[s, r], dst.at[s, r]) for r in cuts for s in range(NS)]
            return dst.at[:, _ds(i * rows, rows, rows)], pairs

        return stream

    def wqb_stream(i):
        cuts = [
            (_ds(i * 16 + lo, 8, 8), pl.ds(col, 2048))
            for lo in (0, 8)
            for col in (0, 2048)
        ]
        pairs = [(wqb_hbm.at[s, *r], wqb.at[s, *r]) for r in cuts for s in range(NS)]
        return wqb.at[:, _ds(i * 16, 16, 16)], pairs

    def cache(src, dst, sizes):
        def stream(i):
            n, j, slot = i >> 4, i & (NJ - 1), i & (NSLOT - 1)
            pairs = [
                (
                    src.at[n * G + g, _ds(j * KEYS + lo, size, 16)],
                    dst.at[slot, g, pl.ds(lo, size)],
                )
                for lo, size in _cuts(sizes)
                for g in range(G)
            ]
            return dst.at[slot], pairs

        return stream

    def both(make, first, second, sizes):
        return make(*first, sizes[0]), make(*second, sizes[1])

    parts = (
        (T_Q, T_U, (wqb_stream, weight(wqa_hbm, wqa, CUT_NARROW[1]))),
        (T_U, T_C, both(weight, (wuk_hbm, wuk), (wuv_hbm, wuv), CUT_NARROW)),
        (T_C, T_KV, both(weight, (c_hbm.at[0], c.at[0]), (c_hbm.at[1], c.at[1]), CUT_WIDE)),
        (T_KV, T_O, both(cache, (k_hbm, kbuf), (v_hbm, vbuf), CUT_CACHE)),
        (T_O, T_END, both(weight, (woa_hbm, woa), (wob_hbm, wob), CUT_WIDE)),
    )

    def start(part, t):
        first, _, streams = parts[part]
        lists = [stream(t - first)[1] for stream in streams]
        _start_interleaved(lists, sems.at[t & (NSLOT - 1)])

    def wait(part, t):
        first, _, streams = parts[part]
        for stream in streams:
            filled = stream(t - first)[0]
            pltpu.make_async_copy(filled, filled, sems.at[t & (NSLOT - 1)]).wait()

    def run(part, body, carry):
        first, end, _ = parts[part]

        def step(t, carry):
            pl.when(t + LAG < end)(lambda: start(part, t + LAG))
            pl.when(t + LAG >= end)(lambda: start(part + 1, t + LAG))
            wait(part, t)
            return body(t - first, carry)

        return lax.fori_loop(first, end, step, carry)

    start(0, 0)
    xa_copy = pltpu.make_async_copy(xa_hbm, xa, small_sems.at[0])
    xb_copy = pltpu.make_async_copy(xb_hbm, xb, small_sems.at[1])
    xa_copy.start()
    xb_copy.start()
    lax.fori_loop(1, LAG, lambda t, _: start(0, t), None)

    ones = jnp.where(_iota((16, 512), 0) == _iota((16, 512), 1) >> 5, 1.0, 0.0)

    def fill_e(i, carry):
        e_ref[i] = jnp.zeros((128, 512), BF16)
        e_ref[i, _ds(i * 16, 16, 16), :] = ones.astype(BF16)
        return carry

    lax.fori_loop(0, NW, fill_e, None)
    own_head = _iota((NS * BH, 128), 0) & (H - 1) == _iota((NS * BH, 128), 1) & (H - 1)

    def keep_own_head(x):
        return jnp.concatenate(
            [
                jnp.where(own_head, x[:, k:k + 128], 0.0).astype(BF16)
                for k in range(0, x.shape[1], 128)
            ],
            axis=1,
        )

    def contract_latent(w_ref, i):
        spread = keep_own_head(_dot(lhs_ref[...], e_ref[i]))
        return sum(
            _dot(spread[s * BH:(s + 1) * BH], w_ref[s, _ds(i * 512, 512, 512), :])
            for s in range(NS)
        )

    for ref in (qb_ref, qlat_ref, la_ref, ctxl_ref, ctx_ref):
        ref[...] = jnp.zeros(ref.shape, F32)
    xa_copy.wait()
    xb_copy.wait()
    xa_val = xa[...].astype(F32)
    xb_val = xb[...].astype(F32)
    for s in range(NS):
        for b in range(B):
            x = xa_val[b:b + 1, s * 128:(s + 1) * 128]
            lhs_ref[pl.ds(s * BH + b * H, H), :] = jnp.broadcast_to(x, (H, 128)).astype(BF16)
    xb_rows = jnp.concatenate(
        [jnp.broadcast_to(xb_val[b:b + 1], (G, M)) for b in range(B)], axis=0
    ).astype(BF16)
    head_row = _iota((B * G, 128), 0) & (G - 1)

    qa = run(0, lambda i, qa: qa + contract_latent(wqa, i), jnp.zeros((BH, D), F32))
    qa = qa.astype(BF16)

    def queries(i, carry):
        full = jnp.concatenate(
            [_dot(qa, wuk[s, _ds(i * 512, 512, 512), :], NT) for s in range(NS)], axis=0
        )
        qlat_ref[...] += _dot(keep_own_head(full), e_ref[i], NT)
        cols = _ds(i * 512, 512, 512)
        full = sum(
            _dot(xb_rows[:, s * 128:(s + 1) * 128], wqb[s, :, cols]) for s in range(NS)
        )
        q16 = qb_ref[i >> 1]
        for u in range(4):
            q16 = jnp.where(head_row == (i & 1) * 4 + u, full[:, u * D:(u + 1) * D], q16)
        qb_ref[i >> 1] = q16
        return carry

    run(1, queries, None)

    qlat = [
        jnp.concatenate(
            [qlat_ref[pl.ds(s * BH + b * H, H), :] for s in range(NS)], axis=1
        ).astype(BF16)
        for b in range(B)
    ]

    def latents(b, i):
        return jnp.concatenate(
            [c[b, s, _ds(i * 128, 128, 128), :] for s in range(NS)], axis=0
        )

    def a_scores(i, m):
        s = jnp.concatenate([_dot(qlat[b], latents(b, i), NT) for b in range(B)], axis=0)
        sa_ref[i] = s
        for k in range(0, 512, 128):
            m = jnp.maximum(m, s[:, k:k + 128])
        return m

    ma = run(2, a_scores, jnp.full((BH, 128), -jnp.inf, F32))
    ma = jnp.broadcast_to(jnp.max(ma, axis=1, keepdims=True), (BH, 128))

    def a_context(i):
        s = sa_ref[i]
        ps = [jnp.exp((s[:, k:k + 128] - ma) * SCALE) for k in range(0, 512, 128)]
        la_ref[...] += (ps[0] + ps[1]) + (ps[2] + ps[3])
        p = jnp.concatenate(ps, axis=1).astype(BF16)
        for b in range(B):
            rows = slice(b * H, (b + 1) * H)
            ctxl_ref[rows, :] += _dot(p[rows], latents(b, i))

    def a_normalize():
        ctx_lat = ctxl_ref[...] / jnp.sum(la_ref[...], axis=1, keepdims=True)
        for s in range(NS):
            lhs_ref[pl.ds(s * BH, BH), :] = ctx_lat[:, s * 128:(s + 1) * 128].astype(BF16)

    def a_values(i):
        ctx_ref[...] += contract_latent(wuv, i)

    row = _iota((G, 128), 0)
    row_keys = _iota((G, KEYS), 0)

    def b_step(i, carry):
        n, j, slot = i >> 4, i & (NJ - 1), i & (NSLOT - 1)
        block, rows = n & (H // G - 1), _ds((n >> 2) * G, G, G)
        m_old = jnp.where(j == 0, -jnp.inf, carry[0])
        l_old = jnp.where(j == 0, 0.0, carry[1])
        acc = jnp.where(j == 0, 0.0, carry[2])
        q = qb_ref[block, rows, :].astype(BF16)
        s = jnp.zeros((G, KEYS), F32)
        for g in range(G):
            s = jnp.where(row_keys == g, _dot(q, kbuf[slot, g], NT), s)
        halves = [s[:, :128], s[:, 128:]]
        m = jnp.maximum(m_old, jnp.max(jnp.maximum(*halves), axis=1, keepdims=True))
        alpha = jnp.exp((m_old - m) * SCALE)
        ps = [jnp.exp((half - m) * SCALE) for half in halves]
        l = alpha * l_old + (ps[0] + ps[1])
        p = jnp.concatenate(ps, axis=1).astype(BF16)
        acc = alpha * acc
        for g in range(G):
            acc = acc + jnp.where(row == g, _dot(p, vbuf[slot, g]), 0.0)

        @pl.when(j == NJ - 1)
        def _():
            ob_ref[block, rows, :] = acc / jnp.sum(l, axis=1, keepdims=True)

        @pl.when(jnp.logical_and(i < 4 * NW, i & 1 == 0))
        def _():
            pl.when(i < 2 * NW)(lambda: a_context(i >> 1))
            pl.when(i == 2 * NW)(a_normalize)
            pl.when(i >= 2 * NW)(lambda: a_values((i >> 1) - NW))

        return m, l, acc

    zero = jnp.zeros((G, 128), F32)
    run(3, b_step, (zero, zero, zero))

    for s in range(NS):
        oa_ref[s] = jnp.concatenate(
            [ctx_ref[pl.ds(b * H + s * G, G), :] for b in range(B)], axis=0
        )

    def project(s, i, out):
        rows = _ds(i * D, D, D)
        return tuple(
            acc + _dot(jnp.where(head_row == i, o_ref[s], 0.0).astype(BF16), w_ref[s, rows, :])
            for acc, o_ref, w_ref in zip(out, (oa_ref, ob_ref), (woa, wob))
        )

    def start_last():
        lists = [stream(NW - 1)[1] for stream in parts[4][2]]
        for s in range(NS):
            _start_interleaved([pairs[s::NS] for pairs in lists], small_sems.at[s])

    def outputs(i, out):
        pl.when(i + LAG < NW - 1)(lambda: start(4, T_O + i + LAG))
        pl.when(i + LAG == NW - 1)(start_last)
        wait(4, T_O + i)
        for s in range(NS):
            out = project(s, i, out)
        return out

    out = lax.fori_loop(0, NW - 1, outputs, (jnp.zeros((B * G, M), F32),) * 2)
    for s in range(NS):
        for dst in (woa, wob):
            filled = dst.at[s, pl.ds((NW - 1) * D, D)]
            pltpu.make_async_copy(filled, filled, small_sems.at[s]).wait()
        out = project(s, NW - 1, out)
    out = jnp.concatenate(out, axis=1)
    out_ref[...] = jnp.concatenate(
        [jnp.sum(out[b * G:(b + 1) * G], axis=0, keepdims=True) for b in range(B)], axis=0
    ).astype(BF16)


@jax.jit
def pallas_concat_heads__compressed_kv_cla__gqa_block_cached__decode_kernel(
    A_x: jax.Array,
    A_c_kv: jax.Array,
    A_w_q: jax.Array,
    A_w_uk: jax.Array,
    A_w_uv: jax.Array,
    A_w_o: jax.Array,
    B_x: jax.Array,
    B_k_cache: jax.Array,
    B_v_cache: jax.Array,
    B_wq: jax.Array,
    B_wo: jax.Array,
):
    assert A_x.shape == B_x.shape == (B, 1, M)
    assert A_c_kv.shape == (B, SK, DC)
    assert A_w_q.shape == (M, H, D) and A_w_o.shape == (H, D, M)
    assert A_w_uk.shape == A_w_uv.shape == (DC, H, D)
    assert B_k_cache.shape == B_v_cache.shape == (B, H, SK, D)
    assert B_wq.shape == (M, H * D) and B_wo.shape == (H * D, M)
    vmem = pltpu.VMEM
    out = pl.pallas_call(
        _kernel,
        in_specs=[pl.BlockSpec(memory_space=pl.ANY)] * 11,
        out_specs=pl.BlockSpec(memory_space=vmem),
        out_shape=jax.ShapeDtypeStruct((B, 2 * M), BF16),
        scratch_shapes=[
            vmem((B, M), BF16),
            vmem((B, M), BF16),
            vmem((B, NS, SK // NS, DC), BF16),
            vmem((NS, M * H // NS, D), BF16),
            vmem((NS, DC * H // NS, D), BF16),
            vmem((NS, DC * H // NS, D), BF16),
            vmem((NS, H * D // NS, M), BF16),
            vmem((NS, M // NS, H * D), BF16),
            vmem((NS, H * D // NS, M), BF16),
            vmem((NSLOT, G, KEYS, D), BF16),
            vmem((NSLOT, G, KEYS, D), BF16),
            vmem((NW, 128, 512), BF16),
            vmem((NS * BH, 128), BF16),
            vmem((NS * BH, 128), F32),
            vmem((H // G, B * G, D), F32),
            vmem((NW, BH, SK // NW), F32),
            vmem((BH, 128), F32),
            vmem((BH, DC), F32),
            vmem((BH, D), F32),
            vmem((H // G, B * G, D), F32),
            vmem((H // G, B * G, D), F32),
            pltpu.SemaphoreType.DMA((NSLOT,)),
            pltpu.SemaphoreType.DMA((NS,)),
        ],
        compiler_params=pltpu.CompilerParams(
            vmem_limit_bytes=64 * 1024 * 1024,
            disable_bounds_checks=True,
            disable_semaphore_checks=True,
        ),
    )(
        A_x.reshape(B, M),
        A_c_kv.reshape(B, NS, SK // NS, DC),
        A_w_q.reshape(NS, M * H // NS, D),
        A_w_uk.reshape(NS, DC * H // NS, D),
        A_w_uv.reshape(NS, DC * H // NS, D),
        A_w_o.reshape(NS, H * D // NS, M),
        B_x.reshape(B, M),
        B_k_cache.reshape(BH, SK, D),
        B_v_cache.reshape(BH, SK, D),
        B_wq.reshape(NS, M // NS, H * D),
        B_wo.reshape(NS, H * D // NS, M),
    )
    return out.reshape(B, 1, 2 * M)
```

```python
import jax
import jax.numpy as jnp
from jax import lax
from jax.experimental import pallas as pl
from jax.experimental.pallas import tpu as pltpu

B, H, SK, D, M = 2, 32, 4096, 128, 512
DC = 4 * D
BH = B * H
G = 8
KEYS = 256
NJ = SK // KEYS
NS = 4
NW = 8
LAG = 3
NSLOT = 4

T_Q = 0
T_U = T_Q + NW
T_C = T_U + NW
T_KV = T_C + NW
T_O = T_KV + BH // G * NJ
T_END = T_O + NW

CUT_CACHE = ((64, 64, 64, 64), (80, 48, 80, 48))
CUT_NARROW = ((128,) * 4, (64,) * 8)
CUT_WIDE = ((32,) * 4, (16,) * 8)

SCALE = float(D) ** -0.5
NN = (((1,), (0,)), ((), ()))
NT = (((1,), (1,)), ((), ()))
F32 = jnp.float32
BF16 = jnp.bfloat16


def _dot(a, b, dims=NN):
    return lax.dot_general(a, b, dims, preferred_element_type=F32)


def _iota(shape, dim):
    return lax.broadcasted_iota(jnp.int32, shape, dim)


def _ds(start, size, align):
    if isinstance(start, int):
        return pl.ds(start, size)
    return pl.ds(pl.multiple_of(start, align), size)


def _cuts(sizes):
    return [(sum(sizes[:k]), size) for k, size in enumerate(sizes)]


def _start_interleaved(lists, sems):
    order = sorted(
        ((k + 0.5 * (1 - priority)) / len(pairs), priority, k)
        for priority, pairs in enumerate(lists)
        for k in range(len(pairs))
    )
    for _, priority, k in order:
        copy = pltpu.make_async_copy(*lists[priority][k], sems[priority])
        copy.start(priority=priority)


def _wait_filled(regions, sems):
    for region, sem in zip(regions, sems, strict=True):
        pltpu.make_async_copy(region, region, sem).wait()


def _kernel(
    xa_hbm, c_hbm, wqa_hbm, wuk_hbm, wuv_hbm, woa_hbm,
    xb_hbm, k_hbm, v_hbm, wqb_hbm, wob_hbm,
    out_ref,
    xa, xb, c, wqa, wuk, wuv, woa, wqb, wob, kbuf, vbuf,
    e_ref, lhs_ref, qlat_ref, qb_ref, sa_ref, la_ref, ctxl_ref, ctx_ref, oa_ref, ob_ref,
    sems, small_sems,
):
    def weight(src, dst, sizes):
        rows = sum(sizes)

        def stream(i):
            cuts = [_ds(i * rows + lo, size, size) for lo, size in _cuts(sizes)]
            pairs = [(src.at[s, r], dst.at[s, r]) for r in cuts for s in range(NS)]
            return dst.at[:, _ds(i * rows, rows, rows)], pairs

        return stream

    def wqb_stream(i):
        cuts = [
            (_ds(i * 16 + lo, 8, 8), pl.ds(col, 2048))
            for lo in (0, 8)
            for col in (0, 2048)
        ]
        pairs = [(wqb_hbm.at[s, *r], wqb.at[s, *r]) for r in cuts for s in range(NS)]
        return wqb.at[:, _ds(i * 16, 16, 16)], pairs

    def cache(src, dst, sizes):
        def stream(i):
            n, j, slot = i >> 4, i & (NJ - 1), i & (NSLOT - 1)
            pairs = [
                (
                    src.at[n * G + g, _ds(j * KEYS + lo, size, 16)],
                    dst.at[slot, g, pl.ds(lo, size)],
                )
                for lo, size in _cuts(sizes)
                for g in range(G)
            ]
            return dst.at[slot], pairs

        return stream

    def both(make, first, second, sizes):
        return make(*first, sizes[0]), make(*second, sizes[1])

    parts = (
        (T_Q, T_U, (wqb_stream, weight(wqa_hbm, wqa, CUT_NARROW[1]))),
        (T_U, T_C, both(weight, (wuk_hbm, wuk), (wuv_hbm, wuv), CUT_NARROW)),
        (T_C, T_KV, both(weight, (c_hbm.at[0], c.at[0]), (c_hbm.at[1], c.at[1]), CUT_WIDE)),
        (T_KV, T_O, both(cache, (k_hbm, kbuf), (v_hbm, vbuf), CUT_CACHE)),
        (T_O, T_END, both(weight, (woa_hbm, woa), (wob_hbm, wob), CUT_WIDE)),
    )

    def start(part, t):
        first, _, streams = parts[part]
        lists = [stream(t - first)[1] for stream in streams]
        _start_interleaved(lists, [sems.at[t & (NSLOT - 1), p] for p in range(2)])

    def wait(part, t):
        first, _, streams = parts[part]
        regions = [stream(t - first)[0] for stream in streams]
        _wait_filled(regions, [sems.at[t & (NSLOT - 1), p] for p in range(2)])

    def run(part, body, carry):
        first, end, _ = parts[part]

        def step(t, carry):
            pl.when(t + LAG < end)(lambda: start(part, t + LAG))
            pl.when(t + LAG >= end)(lambda: start(part + 1, t + LAG))
            wait(part, t)
            return body(t - first, carry)

        return lax.fori_loop(first, end, step, carry)

    start(0, 0)
    xa_copy = pltpu.make_async_copy(xa_hbm, xa, small_sems.at[0, 0])
    xb_copy = pltpu.make_async_copy(xb_hbm, xb, small_sems.at[0, 1])
    xa_copy.start()
    xb_copy.start()
    lax.fori_loop(1, LAG, lambda t, _: start(0, t), None)

    ones = jnp.where(_iota((16, 512), 0) == _iota((16, 512), 1) >> 5, 1.0, 0.0)

    def fill_e(i, carry):
        e_ref[i] = jnp.zeros((128, 512), BF16)
        e_ref[i, _ds(i * 16, 16, 16), :] = ones.astype(BF16)
        return carry

    lax.fori_loop(0, NW, fill_e, None)
    own_head = _iota((NS * BH, 128), 0) & (H - 1) == _iota((NS * BH, 128), 1) & (H - 1)

    def keep_own_head(x):
        return jnp.concatenate(
            [
                jnp.where(own_head, x[:, k:k + 128], 0.0).astype(BF16)
                for k in range(0, x.shape[1], 128)
            ],
            axis=1,
        )

    def contract_latent(w_ref, i):
        spread = keep_own_head(_dot(lhs_ref[...], e_ref[i]))
        return sum(
            _dot(spread[s * BH:(s + 1) * BH], w_ref[s, _ds(i * 512, 512, 512), :])
            for s in range(NS)
        )

    for ref in (qb_ref, qlat_ref, la_ref, ctxl_ref, ctx_ref):
        ref[...] = jnp.zeros(ref.shape, F32)
    xa_copy.wait()
    xb_copy.wait()
    xa_val = xa[...].astype(F32)
    xb_val = xb[...].astype(F32)
    for s in range(NS):
        for b in range(B):
            x = xa_val[b:b + 1, s * 128:(s + 1) * 128]
            lhs_ref[pl.ds(s * BH + b * H, H), :] = jnp.broadcast_to(x, (H, 128)).astype(BF16)
    xb_rows = jnp.concatenate(
        [jnp.broadcast_to(xb_val[b:b + 1], (G, M)) for b in range(B)], axis=0
    ).astype(BF16)
    head_row = _iota((B * G, 128), 0) & (G - 1)

    qa = run(0, lambda i, qa: qa + contract_latent(wqa, i), jnp.zeros((BH, D), F32))
    qa = qa.astype(BF16)

    def queries(i, carry):
        full = jnp.concatenate(
            [_dot(qa, wuk[s, _ds(i * 512, 512, 512), :], NT) for s in range(NS)], axis=0
        )
        qlat_ref[...] += _dot(keep_own_head(full), e_ref[i], NT)
        cols = _ds(i * 512, 512, 512)
        full = sum(
            _dot(xb_rows[:, s * 128:(s + 1) * 128], wqb[s, :, cols]) for s in range(NS)
        )
        q16 = qb_ref[i >> 1]
        for u in range(4):
            q16 = jnp.where(head_row == (i & 1) * 4 + u, full[:, u * D:(u + 1) * D], q16)
        qb_ref[i >> 1] = q16
        return carry

    run(1, queries, None)

    qlat = [
        jnp.concatenate(
            [qlat_ref[pl.ds(s * BH + b * H, H), :] for s in range(NS)], axis=1
        ).astype(BF16)
        for b in range(B)
    ]

    def latents(b, i):
        return jnp.concatenate(
            [c[b, s, _ds(i * 128, 128, 128), :] for s in range(NS)], axis=0
        )

    def a_scores(i, m):
        s = jnp.concatenate([_dot(qlat[b], latents(b, i), NT) for b in range(B)], axis=0)
        sa_ref[i] = s
        for k in range(0, 512, 128):
            m = jnp.maximum(m, s[:, k:k + 128])
        return m

    ma = run(2, a_scores, jnp.full((BH, 128), -jnp.inf, F32))
    ma = jnp.broadcast_to(jnp.max(ma, axis=1, keepdims=True), (BH, 128))

    def a_context(i):
        s = sa_ref[i]
        ps = [jnp.exp((s[:, k:k + 128] - ma) * SCALE) for k in range(0, 512, 128)]
        la_ref[...] += (ps[0] + ps[1]) + (ps[2] + ps[3])
        p = jnp.concatenate(ps, axis=1).astype(BF16)
        for b in range(B):
            rows = slice(b * H, (b + 1) * H)
            ctxl_ref[rows, :] += _dot(p[rows], latents(b, i))

    def a_normalize():
        ctx_lat = ctxl_ref[...] / jnp.sum(la_ref[...], axis=1, keepdims=True)
        for s in range(NS):
            lhs_ref[pl.ds(s * BH, BH), :] = ctx_lat[:, s * 128:(s + 1) * 128].astype(BF16)

    def a_values(i):
        ctx_ref[...] += contract_latent(wuv, i)

    row = _iota((G, 128), 0)
    row_keys = _iota((G, KEYS), 0)

    def b_step(i, carry):
        n, j, slot = i >> 4, i & (NJ - 1), i & (NSLOT - 1)
        block, rows = n & (H // G - 1), _ds((n >> 2) * G, G, G)
        m_old = jnp.where(j == 0, -jnp.inf, carry[0])
        l_old = jnp.where(j == 0, 0.0, carry[1])
        acc = jnp.where(j == 0, 0.0, carry[2])
        q = qb_ref[block, rows, :].astype(BF16)
        s = jnp.zeros((G, KEYS), F32)
        for g in range(G):
            s = jnp.where(row_keys == g, _dot(q, kbuf[slot, g], NT), s)
        halves = [s[:, :128], s[:, 128:]]
        m = jnp.maximum(m_old, jnp.max(jnp.maximum(*halves), axis=1, keepdims=True))
        alpha = jnp.exp((m_old - m) * SCALE)
        ps = [jnp.exp((half - m) * SCALE) for half in halves]
        l = alpha * l_old + (ps[0] + ps[1])
        p = jnp.concatenate(ps, axis=1).astype(BF16)
        acc = alpha * acc
        for g in range(G):
            acc = acc + jnp.where(row == g, _dot(p, vbuf[slot, g]), 0.0)

        @pl.when(j == NJ - 1)
        def _():
            ob_ref[block, rows, :] = acc / jnp.sum(l, axis=1, keepdims=True)

        @pl.when(jnp.logical_and(i < 4 * NW, i & 1 == 0))
        def _():
            pl.when(i < 2 * NW)(lambda: a_context(i >> 1))
            pl.when(i == 2 * NW)(a_normalize)
            pl.when(i >= 2 * NW)(lambda: a_values((i >> 1) - NW))

        return m, l, acc

    zero = jnp.zeros((G, 128), F32)
    run(3, b_step, (zero, zero, zero))

    for s in range(NS):
        oa_ref[s] = jnp.concatenate(
            [ctx_ref[pl.ds(b * H + s * G, G), :] for b in range(B)], axis=0
        )

    def project(s, i, out):
        rows = _ds(i * D, D, D)
        return tuple(
            acc + _dot(jnp.where(head_row == i, o_ref[s], 0.0).astype(BF16), w_ref[s, rows, :])
            for acc, o_ref, w_ref in zip(out, (oa_ref, ob_ref), (woa, wob))
        )

    def start_last():
        lists = [stream(NW - 1)[1] for stream in parts[4][2]]
        for s in range(NS):
            head = [pairs[s::NS] for pairs in lists]
            _start_interleaved(head, [small_sems.at[s, p] for p in range(2)])

    def outputs(i, out):
        pl.when(i + LAG < NW - 1)(lambda: start(4, T_O + i + LAG))
        pl.when(i + LAG == NW - 1)(start_last)
        wait(4, T_O + i)
        for s in range(NS):
            out = project(s, i, out)
        return out

    out = lax.fori_loop(0, NW - 1, outputs, (jnp.zeros((B * G, M), F32),) * 2)
    for s in range(NS):
        regions = [dst.at[s, pl.ds((NW - 1) * D, D)] for dst in (woa, wob)]
        _wait_filled(regions, [small_sems.at[s, p] for p in range(2)])
        out = project(s, NW - 1, out)
    out = jnp.concatenate(out, axis=1)
    out_ref[...] = jnp.concatenate(
        [jnp.sum(out[b * G:(b + 1) * G], axis=0, keepdims=True) for b in range(B)], axis=0
    ).astype(BF16)


@jax.jit
def pallas_concat_heads__compressed_kv_cla__gqa_block_cached__decode_kernel(
    A_x: jax.Array,
    A_c_kv: jax.Array,
    A_w_q: jax.Array,
    A_w_uk: jax.Array,
    A_w_uv: jax.Array,
    A_w_o: jax.Array,
    B_x: jax.Array,
    B_k_cache: jax.Array,
    B_v_cache: jax.Array,
    B_wq: jax.Array,
    B_wo: jax.Array,
):
    assert A_x.shape == B_x.shape == (B, 1, M)
    assert A_c_kv.shape == (B, SK, DC)
    assert A_w_q.shape == (M, H, D) and A_w_o.shape == (H, D, M)
    assert A_w_uk.shape == A_w_uv.shape == (DC, H, D)
    assert B_k_cache.shape == B_v_cache.shape == (B, H, SK, D)
    assert B_wq.shape == (M, H * D) and B_wo.shape == (H * D, M)
    vmem = pltpu.VMEM
    out = pl.pallas_call(
        _kernel,
        in_specs=[pl.BlockSpec(memory_space=pl.ANY)] * 11,
        out_specs=pl.BlockSpec(memory_space=vmem),
        out_shape=jax.ShapeDtypeStruct((B, 2 * M), BF16),
        scratch_shapes=[
            vmem((B, M), BF16),
            vmem((B, M), BF16),
            vmem((B, NS, SK // NS, DC), BF16),
            vmem((NS, M * H // NS, D), BF16),
            vmem((NS, DC * H // NS, D), BF16),
            vmem((NS, DC * H // NS, D), BF16),
            vmem((NS, H * D // NS, M), BF16),
            vmem((NS, M // NS, H * D), BF16),
            vmem((NS, H * D // NS, M), BF16),
            vmem((NSLOT, G, KEYS, D), BF16),
            vmem((NSLOT, G, KEYS, D), BF16),
            vmem((NW, 128, 512), BF16),
            vmem((NS * BH, 128), BF16),
            vmem((NS * BH, 128), F32),
            vmem((H // G, B * G, D), F32),
            vmem((NW, BH, SK // NW), F32),
            vmem((BH, 128), F32),
            vmem((BH, DC), F32),
            vmem((BH, D), F32),
            vmem((H // G, B * G, D), F32),
            vmem((H // G, B * G, D), F32),
            pltpu.SemaphoreType.DMA((NSLOT, 2)),
            pltpu.SemaphoreType.DMA((NS, 2)),
        ],
        compiler_params=pltpu.CompilerParams(
            vmem_limit_bytes=64 * 1024 * 1024,
            disable_bounds_checks=True,
            disable_semaphore_checks=True,
        ),
    )(
        A_x.reshape(B, M),
        A_c_kv.reshape(B, NS, SK // NS, DC),
        A_w_q.reshape(NS, M * H // NS, D),
        A_w_uk.reshape(NS, DC * H // NS, D),
        A_w_uv.reshape(NS, DC * H // NS, D),
        A_w_o.reshape(NS, H * D // NS, M),
        B_x.reshape(B, M),
        B_k_cache.reshape(BH, SK, D),
        B_v_cache.reshape(BH, SK, D),
        B_wq.reshape(NS, M // NS, H * D),
        B_wo.reshape(NS, H * D // NS, M),
    )
    return out.reshape(B, 1, 2 * M)
```
